```python
import jax
import jax.numpy as jnp

def _softmax(x, axis=-1):
    return jax.nn.softmax(x, axis=axis)
def _gelu(x):
    return jax.nn.gelu(x, approximate=True)
def _silu(x):
    return jax.nn.silu(x)
def _sigmoid(x):
    return jax.nn.sigmoid(x)
def _layernorm(x, axis=-1, eps=1e-5):
    m = jnp.mean(x, axis=axis, keepdims=True)
    v = jnp.var(x, axis=axis, keepdims=True)
    return (x - m) / jnp.sqrt(v + eps)
def _scatter_add(tgt, idx, src, axis=0):
    return tgt.at[idx].add(src)
def _segment_sum(src, seg, n):
    return jax.ops.segment_sum(src, seg, n)
class _Rng:
    def __init__(self, key):
        self._k = key
    def _next(self):
        self._k, sub = jax.random.split(self._k)
        return sub
    def normal(self, shape):
        return jax.random.normal(self._next(), shape, dtype=jnp.bfloat16)
    def randint(self, lo, hi, shape):
        return jax.random.randint(self._next(), shape, lo, hi, dtype=jnp.int32)
    def uniform(self, shape, lo=0.0, hi=1.0):
        return jax.random.uniform(self._next(), shape, jnp.bfloat16, lo, hi)
    def permutation(self, n):
        return jax.random.permutation(self._next(), n)


kernel_name = 'parallel_sum__compressed_kv_cla__moe_arch_mod__prompt'

def setup_inputs():
    _rng = _Rng(jax.random.key(int.from_bytes(__import__("os").urandom(4), "little")))
    _w = (lambda a: (lambda t: t.astype(jnp.bfloat16) if jnp.issubdtype(t.dtype, jnp.floating) else t)(jnp.asarray(a)))
    def _A_setup():
        B, H, Sq, Sk, D, M = 1, 32, 2048, 2048, 128, 640
        Dc = 4 * D
        return {
            "x": _w((lambda *s: _rng.normal(s) * 0.05)(B, Sq, M)),
            "c_kv": _w((lambda *s: _rng.normal(s) * 0.05)(B, Sk, Dc)),
            "w_q": _w((lambda *s: _rng.normal(s) * 0.05)(M, H, D) * (M ** -0.5)),
            "w_uk": _w((lambda *s: _rng.normal(s) * 0.05)(Dc, H, D) * (Dc ** -0.5)),
            "w_uv": _w((lambda *s: _rng.normal(s) * 0.05)(Dc, H, D) * (Dc ** -0.5)),
            "w_o": _w((lambda *s: _rng.normal(s) * 0.05)(H, D, M) * ((H * D) ** -0.5)),
        }
    _A_in = _A_setup()

    def _B_setup():
        B, S, D, F, C = 1, 2048, 640, 1728, 8
        return {
            "x": _w((lambda *s: _rng.normal(s) * 0.05)(B, S, D)),
            "w_r": _w((lambda *s: _rng.normal(s) * 0.05)(D)),
            "w_gate": _w((lambda *s: _rng.normal(s) * 0.05)(D, F)),
            "w_up": _w((lambda *s: _rng.normal(s) * 0.05)(D, F)),
            "w_down": _w((lambda *s: _rng.normal(s) * 0.05)(F, D)),
        }
    _B_in = _B_setup()

    return {
        "A_x": _A_in["x"],
        "A_c_kv": _A_in["c_kv"],
        "A_w_q": _A_in["w_q"],
        "A_w_uk": _A_in["w_uk"],
        "A_w_uv": _A_in["w_uv"],
        "A_w_o": _A_in["w_o"],
        "B_x": _B_in["x"],
        "B_w_r": _B_in["w_r"],
        "B_w_gate": _B_in["w_gate"],
        "B_w_up": _B_in["w_up"],
        "B_w_down": _B_in["w_down"],
    }

def reference(A_x, A_c_kv, A_w_q, A_w_uk, A_w_uv, A_w_o, B_x, B_w_r, B_w_gate, B_w_up, B_w_down):
    def _A_ref(x, c_kv, w_q, w_uk, w_uv, w_o):
        B, Sq, M = x.shape[0], x.shape[1], x.shape[2]
        Sk = c_kv.shape[1]
        H, D = w_q.shape[1], w_q.shape[2]
        q = jnp.einsum("bqm,mhd->bhqd", x, w_q)
        k = jnp.einsum("bkc,chd->bhkd", c_kv, w_uk)
        v = jnp.einsum("bkc,chd->bhkd", c_kv, w_uv)
        scores = jnp.einsum("bhqd,bhkd->bhqk", q, k) * (D ** -0.5)
        off = Sk - Sq
        qi = jnp.arange(Sq)[:, None]
        kj = jnp.arange(Sk)[None, :]
        cmask = kj <= (qi + off)
        scores = jnp.where(cmask[None, None], scores, -1e9)
        p = _softmax(scores, axis=-1)
        ctx = jnp.einsum("bhqk,bhkd->bhqd", p, v)
        return jnp.einsum("bhqd,hdm->bqm", ctx, w_o)

    def _B_ref(x, w_r, w_gate, w_up, w_down):
        B, S, D = x.shape
        C = 8
        r = x @ w_r
        idx = jnp.argsort(-r, axis=-1)[:, :C]
        idx_e = jnp.repeat(idx.reshape(B, C, 1), D, axis=2)
        x_sel = jnp.take_along_axis(x, idx_e, axis=1)
        g = _silu(x_sel @ w_gate)
        u = x_sel @ w_up
        y = (g * u) @ w_down
        r_sel = _sigmoid(jnp.take_along_axis(r, idx, axis=1))
        y = y * r_sel.reshape(B, C, 1)
        b_off = (jnp.arange(B) * S).reshape(B, 1)
        flat_idx = (idx + b_off).reshape(B * C)
        zero = (x * 0.0).reshape(B * S, D)
        upd = _scatter_add(zero, flat_idx, y.reshape(B * C, D), axis=0)
        return x + upd.reshape(B, S, D)

    x = A_x
    xn = _layernorm(x, axis=-1)
    return x + _A_ref(xn, A_c_kv, A_w_q, A_w_uk, A_w_uv, A_w_o) + _B_ref(xn, B_w_r, B_w_gate, B_w_up, B_w_down)
```

```python
import functools, math
import jax
import jax.numpy as jnp
from jax import lax
import jax.experimental.pallas as pl
import jax.experimental.pallas.tpu as pltpu

BF = jnp.bfloat16
F32 = jnp.float32
U32 = jnp.uint32
I32 = jnp.int32
NT = (((1,), (1,)), ((), ()))
T = 128
HT = T // 2
R = 512
HR = R // 2
LAG = 40
CAP = 8

def _dot(a, b):
    return jnp.dot(a, b, preferred_element_type=F32)

def _dot_nt(a, b):
    return lax.dot_general(a, b, NT, preferred_element_type=F32)

def _pk(x):
    return pltpu.bitcast(x.astype(BF), U32)

def _up(x):
    return pltpu.bitcast(x, BF)

def _rb(x):
    return x.astype(BF).astype(F32)

def _unpair(w32):
    lo = pltpu.bitcast(w32 << 16, F32)
    hi = pltpu.bitcast(w32 & jnp.uint32(0xFFFF0000), F32)
    return lo, hi

def kernel(x_hbm, c_hbm, wq_hbm, wk_hbm, wv_hbm, wo_hbm, wr_ref, wg_hbm, wu_hbm, wd_hbm, o_hbm,
           x_ref, xn_ref, cs_ref, acc_ref, q_ref, k_ref, vt_ref, ctx_ref,
           rq_ref, rk_ref, rv_ref, wo_ref, wq_ref, wk_ref, wvt_ref, ffn_ref, xs_ref, y_ref, idx_ref,
           s_w, s_o, s_f, s_x, s_c, *, S, M, D, NP, FD):
    scale = (D ** -0.5) * math.log2(math.e)
    NM = M // T
    NC = cs_ref.shape[0]
    NS = S // T
    NR = S // R

    def w_copies(p):
        return [pltpu.make_async_copy(h.bitcast(U32).at[:, p, 0, :], b.at[p % 2], s_w.at[p % 2 * 3 + i])
                for i, (h, b) in enumerate(((wk_hbm, rk_ref), (wv_hbm, rv_ref), (wq_hbm, rq_ref)))]

    def wo_copy(p):
        return pltpu.make_async_copy(wo_hbm.bitcast(U32).at[p], wo_ref.at[p % 2], s_o.at[p % 2])

    def f_start(p):
        return jnp.minimum(p * T, FD - T)

    def f_copies(p):
        rows = pl.ds(pl.multiple_of(f_start(p) // 2, 32), HT)
        return [pltpu.make_async_copy(h.bitcast(U32).at[rows, :], ffn_ref.at[p % 2, i], s_f.at[p % 2 * 3 + i])
                for i, h in enumerate((wg_hbm, wu_hbm, wd_hbm))]

    def x_copy(r):
        return pltpu.make_async_copy(x_hbm.at[0, r * R:(r + 1) * R, :], x_ref.at[r * R:(r + 1) * R, :], s_x.at[r])

    def c_copies(r):
        return [pltpu.make_async_copy(c_hbm.bitcast(U32).at[0, r * HR:(r + 1) * HR, t * T:(t + 1) * T],
                                      cs_ref.at[t, r * HR:(r + 1) * HR, :], s_c.at[r * NC + t]) for t in range(NC)]

    def o_copy(r):
        return pltpu.make_async_copy(x_ref.at[r * R:(r + 1) * R, :], o_hbm.at[0, r * R:(r + 1) * R, :], s_x.at[r])

    def prep_k(p):
        a, b = _unpair(rk_ref[p % 2])
        wk_ref[:, :T] = _pk(a)
        wk_ref[:, T:] = _pk(b)

    def prep_q(p):
        a, b = _unpair(rq_ref[p % 2])
        wq_ref[:, :T] = _pk(a)
        wq_ref[:, T:] = _pk(b)

    def prep_v(p):
        a, b = _unpair(rv_ref[p % 2])
        wvt_ref[:HT, :] = _pk(a.T)
        wvt_ref[HT:, :] = _pk(b.T)

    def proj_k(r):
        rs = slice(r * HR, (r + 1) * HR)
        cc = jnp.concatenate([_up(cs_ref[t, rs, :]) for t in range(NC)], axis=1)
        kk = _dot(cc, _up(wk_ref[...]))
        k_ref[0, rs, :] = _pk(kk[:, :T])
        k_ref[1, rs, :] = _pk(kk[:, T:])

    def proj_q(r):
        rs = slice(r * HR, (r + 1) * HR)
        xx = jnp.concatenate([_up(xn_ref[t, rs, :]) for t in range(NM)], axis=1)
        qq = _dot(xx, _up(wq_ref[...])) * scale
        q_ref[0, rs, :] = _pk(qq[:, :T])
        q_ref[1, rs, :] = _pk(qq[:, T:])

    def proj_v(s):
        rs = slice(s * HT, (s + 1) * HT)
        cc = jnp.concatenate([_up(cs_ref[t, rs, :]) for t in range(NC)], axis=1)
        vv = _dot_nt(_up(wvt_ref[...]), cc)
        vt_ref[0, s] = _pk(vv[:T])
        vt_ref[1, s] = _pk(vv[T:])

    def layernorm(s):
        x = x_ref[s * T:(s + 1) * T, :].astype(F32)
        m = jnp.sum(x, axis=-1, keepdims=True) * (1.0 / M)
        d = x - m
        v = jnp.sum(d * d, axis=-1, keepdims=True) * (1.0 / M)
        den = _rb(jnp.sqrt(_rb(_rb(v) + 1e-5)))
        xn = (_rb(x - _rb(m)) * (1.0 / den)).astype(BF)
        for t in range(NM):
            xn_ref[t, s * HT:(s + 1) * HT, :] = pltpu.bitcast(xn[:, t * T:(t + 1) * T], U32)
        return xn

    def attention():
        key = lax.broadcasted_iota(I32, (T, T), 0)
        qry = lax.broadcasted_iota(I32, (T, T), 1)
        tri = key <= qry
        tiles = [(h, i, j) for h in range(2) for i in range(NS) for j in range(i + 1)]
        sval, mx, mfin, lsum, oacc = {}, {}, {}, {}, {}

        def qk(h, i, j):
            s = _dot_nt(_up(k_ref[h, j * HT:(j + 1) * HT, :]), _up(q_ref[h, i * HT:(i + 1) * HT, :]))
            if j == i:
                s = jnp.where(tri, s, -1e9)
            sval[h, i, j] = s
            m8 = jnp.max(s.reshape(T // 8, 8, T), axis=0)
            mx[h, i] = m8 if j == 0 else jnp.maximum(mx[h, i], m8)
            if j == i:
                mfin[h, i] = jnp.max(mx[h, i], axis=0, keepdims=True)

        def pv(h, i, j):
            p = jnp.exp2(sval.pop((h, i, j)) - mfin[h, i])
            l8 = jnp.sum(p.reshape(T // 8, 8, T), axis=0)
            lsum[h, i] = l8 if j == 0 else lsum[h, i] + l8
            o = _dot(_up(vt_ref[h, j]), p.astype(BF))
            oacc[h, i] = o if j == 0 else oacc[h, i] + o
            if j == i:
                l = jnp.sum(lsum[h, i], axis=0, keepdims=True)
                ctx_ref[h, i * HT:(i + 1) * HT, :] = _pk((oacc[h, i] * (1.0 / l)).T)

        n = len(tiles)
        for t in range(n + LAG):
            if t < n:
                qk(*tiles[t])
            if t >= LAG:
                pv(*tiles[t - LAG])

    def out_proj(p, r):
        rs = slice(r * HR, (r + 1) * HR)
        cc = jnp.concatenate([_up(ctx_ref[0, rs, :]), _up(ctx_ref[1, rs, :])], axis=1)
        return _dot(cc, _up(wo_ref[p % 2]))

    wk0, wv0, wq0 = w_copies(0)
    wk0.start()
    for r in range(NR):
        for cp in c_copies(r):
            cp.start()
    wv0.start()
    for r in range(NR):
        x_copy(r).start()
    wq0.start()
    wo_copy(0).start()
    for cp in f_copies(0):
        cp.start()
    acc_ref[...] = jnp.zeros(acc_ref.shape, F32)
    y_ref[...] = jnp.zeros(y_ref.shape, F32)
    wk0.wait()
    prep_k(0)
    for r in range(NR):
        for cp in c_copies(r):
            cp.wait()
        proj_k(r)
        if r == 1:
            wv0.wait()
            prep_v(0)
    wr = jnp.broadcast_to(wr_ref[...].reshape(1, M), (NS, M))
    sub = lax.broadcasted_iota(I32, (NS, T), 0)
    score = jnp.zeros((NS, T), F32)
    for s in range(NS):
        if s % (R // T) == 0:
            x_copy(s // (R // T)).wait()
        proj_v(s)
        xn = layernorm(s)
        score = jnp.where(sub == s, _dot_nt(wr, xn), score)
    wq0.wait()
    prep_q(0)
    for cp in w_copies(1):
        cp.start()

    score = _rb(score)
    key = jnp.where(score != score, -jnp.inf, score)
    pos = sub * T + lax.broadcasted_iota(I32, (NS, T), 1)
    row8 = lax.broadcasted_iota(I32, (CAP, T), 0)
    gate = jnp.zeros((CAP, T), F32)
    xs = [jnp.zeros((CAP, T), F32) for _ in range(NM)]
    for i in range(CAP):
        best = jnp.max(jnp.max(key, axis=1, keepdims=True), axis=0, keepdims=True)
        cand = jnp.where(key == best, pos, S)
        sel = jnp.min(jnp.min(cand, axis=1, keepdims=True), axis=0, keepdims=True)
        hit = pos == sel
        key = jnp.where(hit, -jnp.inf, key)
        pos = jnp.where(hit, S, pos)
        gate = jnp.where(row8 == i, best, gate)
        tok = jnp.minimum(sel[0, 0], S - 1)
        idx_ref[i] = tok
        sh = ((1 - tok % 2) * 16).astype(U32)
        for t in range(NM):
            w = xn_ref[t, pl.ds(tok // 2, 1), :]
            row = pltpu.bitcast((w << sh) & jnp.uint32(0xFFFF0000), F32)
            xs[t] = jnp.where(row8 == i, row, xs[t])
        if i % 2 == 1:
            proj_q(i // 2 * NR // 4) if NR == 4 else None
    xs_ref[...] = jnp.concatenate(xs, axis=1)
    gate = _rb(1.0 / (1.0 + jnp.exp(-gate)))

    def body(p, carry):
        wo_copy(p).wait()
        for cp in f_copies(p) + w_copies(p + 1):
            cp.wait()
        wo_copy(p + 1).start()

        @pl.when(p + 2 < NP)
        def _():
            for cp in f_copies(p + 1) + w_copies(p + 2):
                cp.start()
        xsel = xs_ref[...].astype(BF)
        g = _rb(_dot_nt(xsel, _up(ffn_ref[p % 2, 0])))
        u = _rb(_dot_nt(xsel, _up(ffn_ref[p % 2, 1])))
        prep_k(p + 1)
        prep_v(p + 1)
        prep_q(p + 1)
        attention()
        hcol = f_start(p) + lax.broadcasted_iota(I32, (CAP, T), 1)
        hid = jnp.where(hcol >= p * T, _rb(g / (1.0 + jnp.exp(-g))) * u, 0.0).astype(BF)
        y_ref[...] += _dot(hid, _up(ffn_ref[p % 2, 2]))
        for r in range(NR):
            oo = out_proj(p, r)
            for t in range(NM):
                acc_ref[t, r * R:(r + 1) * R, :] += oo[:, t * T:(t + 1) * T]
        for s in range(NS):
            proj_v(s)
        for r in range(NR):
            proj_k(r)
        for r in range(NR):
            proj_q(r)
        return carry

    lax.fori_loop(0, NP - 1, body, 0)

    wo_copy(NP - 1).wait()
    y = _rb(_rb(y_ref[...]) * gate[:, :1])
    for i in range(CAP):
        tok = idx_ref[i]
        for t in range(NM):
            acc_ref[t, pl.ds(tok, 1), :] += y[i:i + 1, t * T:(t + 1) * T]
    attention()
    for r in range(NR):
        oo = out_proj(NP - 1, r)
        for t in range(NM):
            rows = slice(r * R, (r + 1) * R)
            base = x_ref[rows, t * T:(t + 1) * T].astype(F32) + _up(xn_ref[t, r * HR:(r + 1) * HR, :]).astype(F32)
            x_ref[rows, t * T:(t + 1) * T] = (base + (acc_ref[t, rows, :] + oo[:, t * T:(t + 1) * T])).astype(BF)
        o_copy(r).start()
    for r in range(NR):
        o_copy(r).wait()

@jax.jit
def pallas_parallel_sum__compressed_kv_cla__moe_arch_mod__prompt_kernel(
    A_x, A_c_kv, A_w_q, A_w_uk, A_w_uv, A_w_o, B_x, B_w_r, B_w_gate, B_w_up, B_w_down):
    B, S, M = A_x.shape
    Dc = A_c_kv.shape[2]
    H, D = A_w_q.shape[1:]
    FD = B_w_gate.shape[1]
    NP = H // 2
    hbm = pl.BlockSpec(memory_space=pltpu.HBM)
    dma = pltpu.SemaphoreType.DMA
    out = pl.pallas_call(
        functools.partial(kernel, S=S, M=M, D=D, NP=NP, FD=FD),
        in_specs=[hbm] * 6 + [pl.BlockSpec(memory_space=pltpu.VMEM)] + [hbm] * 3,
        out_specs=hbm,
        out_shape=jax.ShapeDtypeStruct((B, S, M), BF),
        scratch_shapes=[
            pltpu.VMEM((S, M), BF),
            pltpu.VMEM((M // T, S // 2, T), U32), pltpu.VMEM((Dc // T, S // 2, T), U32), pltpu.VMEM((M // T, S, T), F32),
            pltpu.VMEM((2, S // 2, D), U32), pltpu.VMEM((2, S // 2, D), U32), pltpu.VMEM((2, S // T, D // 2, T), U32),
            pltpu.VMEM((2, S // 2, D), U32),
            pltpu.VMEM((2, M, D), U32), pltpu.VMEM((2, Dc, D), U32), pltpu.VMEM((2, Dc, D), U32), pltpu.VMEM((2, D, M), U32),
            pltpu.VMEM((M // 2, 2 * D), U32), pltpu.VMEM((Dc // 2, 2 * D), U32), pltpu.VMEM((D, Dc), U32),
            pltpu.VMEM((2, 3, HT, M), U32), pltpu.VMEM((CAP, M), F32), pltpu.VMEM((CAP, M), F32), pltpu.SMEM((CAP,), I32),
            dma((6,)), dma((2,)), dma((6,)), dma((S // R,)), dma((S // R * (Dc // T),)),
        ],
        compiler_params=pltpu.CompilerParams(vmem_limit_bytes=120 * 2**20),
    )(A_x, A_c_kv, A_w_q.reshape(M, NP, 2, D), A_w_uk.reshape(Dc, NP, 2, D), A_w_uv.reshape(Dc, NP, 2, D),
      A_w_o.reshape(NP, 2 * D, M), B_w_r, B_w_gate.T, B_w_up.T, B_w_down)
    return out
```

```python
import functools, math
import jax
import jax.numpy as jnp
from jax import lax
import jax.experimental.pallas as pl
import jax.experimental.pallas.tpu as pltpu

BF = jnp.bfloat16
F32 = jnp.float32
U32 = jnp.uint32
I32 = jnp.int32
NT = (((1,), (1,)), ((), ()))
T = 128
HT = T // 2
R = 512
HR = R // 2
LAG = 40
VI = 2
CAP = 8
Q0 = 24
FC = 256
CUTS = [0,1280,1792,2048]
NB = True
PIN = 1

def _dot(a, b):
    return jnp.dot(a, b, preferred_element_type=F32)

def _dot_nt(a, b):
    return lax.dot_general(a, b, NT, preferred_element_type=F32)

def _pk(x):
    return pltpu.bitcast(x.astype(BF), U32)

def _up(x):
    return pltpu.bitcast(x, BF)

def _rb(x):
    return x.astype(BF).astype(F32)

def _half(w32, odd):
    sh = ((1 - odd) * 16).astype(U32)
    return pltpu.bitcast((w32 << sh) & jnp.uint32(0xFFFF0000), F32)

def kernel(x_hbm, c_hbm, wq_hbm, wk_hbm, wv_hbm, wo_hbm, wr_ref, wg_hbm, wu_hbm, wd_hbm, o_hbm,
           x_ref, xn_ref, cs_ref, acc_ref, q_ref, k_ref, vt_ref, ctx_ref,
           rq_ref, rk_ref, rv_ref, wo_ref, wq_ref, wk_ref, wvt_ref, ffn_ref, xs_ref, y_ref, idx_ref,
           s_w, s_o, s_f, s_x, s_c, *, S, M, D, H, FD):
    scale = (D ** -0.5) * math.log2(math.e)
    NM = M // T
    NS = S // T
    NR = S // R

    def w_copies(h):
        return [pltpu.make_async_copy(w.bitcast(U32).at[:, jnp.minimum(h, H - 1) >> 1, 0, :], b.at[h & 1], s_w.at[(h & 1) * 3 + i])
                for i, (w, b) in enumerate(((wk_hbm, rk_ref), (wv_hbm, rv_ref), (wq_hbm, rq_ref)))]

    def wo_copy(h):
        return pltpu.make_async_copy(wo_hbm.bitcast(U32).at[jnp.minimum(h, H - 1)], wo_ref.at[h & 1], s_o.at[h & 1])

    def f_start(h):
        return jnp.minimum((h - 1) * T, FD - T)

    def f_copies(h):
        rows = pl.ds(pl.multiple_of(f_start(h) >> 1, 32), HT)
        return [pltpu.make_async_copy(w.bitcast(U32).at[rows, :], ffn_ref.at[h & 1, i], s_f.at[(h & 1) * 3 + i])
                for i, w in enumerate((wg_hbm, wu_hbm, wd_hbm))]

    def x_copy(r):
        return pltpu.make_async_copy(x_hbm.at[0, r * R:(r + 1) * R, :], x_ref.at[r * R:(r + 1) * R, :], s_x.at[r])

    def c_copies(r):
        rs = slice(r * HR, (r + 1) * HR)
        return [pltpu.make_async_copy(c_hbm.bitcast(U32).at[0, rs, :], cs_ref.at[rs, :], s_c.at[r])]

    def o_copy(k, lo, hi):
        return pltpu.make_async_copy(x_ref.at[lo:hi, :], o_hbm.at[0, lo:hi, :], s_x.at[k])

    def prep_k(h):
        wk_ref[...] = _pk(_half(rk_ref[h & 1], h & 1))

    def prep_q(h):
        wq_ref[...] = _pk(_half(rq_ref[h & 1], h & 1))

    def prep_v(h):
        wvt_ref[...] = _pk(_half(rv_ref[h & 1], h & 1).T)

    def proj_k(r):
        rs = slice(r * HR, (r + 1) * HR)
        cc = _up(cs_ref[rs, :])
        k_ref[rs, :] = _pk(_dot(cc, _up(wk_ref[...])))

    def proj_q(r):
        rs = slice(r * HR, (r + 1) * HR)
        xx = jnp.concatenate([_up(xn_ref[t, rs, :]) for t in range(NM)], axis=1)
        q_ref[rs, :] = _pk(_dot(xx, _up(wq_ref[...])) * scale)

    def proj_v(s):
        rs = slice(s * HT, (s + 1) * HT)
        cc = _up(cs_ref[rs, :])
        vt_ref[s] = _pk(_dot_nt(_up(wvt_ref[...]), cc))

    def layernorm(s):
        x = x_ref[s * T:(s + 1) * T, :].astype(F32)
        m = jnp.sum(x, axis=-1, keepdims=True) * (1.0 / M)
        d = x - m
        v = jnp.sum(d * d, axis=-1, keepdims=True) * (1.0 / M)
        den = _rb(jnp.sqrt(_rb(_rb(v) + 1e-5)))
        xn = (_rb(x - _rb(m)) * (1.0 / den)).astype(BF)
        for t in range(NM):
            xn_ref[t, s * HT:(s + 1) * HT, :] = pltpu.bitcast(xn[:, t * T:(t + 1) * T], U32)
        return xn

    tiles = [(i, j) for i in range(NS) for j in range(i + 1)]
    NTL = len(tiles)

    def first(i):
        return i * (i + 1) // 2

    def attention():
        key = lax.broadcasted_iota(I32, (T, T), 0)
        qry = lax.broadcasted_iota(I32, (T, T), 1)
        tri = key <= qry
        sval, mx, mfin, lsum, oacc, hist = {}, {}, {}, {}, {}, []

        def qk(n):
            i, j = tiles[n]
            s = _dot_nt(_up(k_ref[j * HT:(j + 1) * HT, :]), _up(q_ref[i * HT:(i + 1) * HT, :]))
            if j == i:
                s = jnp.where(tri, s, -1e9)
            sval[i, j] = s
            m8 = jnp.max(s.reshape(T // 8, 8, T), axis=0)
            mx[i] = m8 if j == 0 else jnp.maximum(mx[i], m8)
            if j == i:
                mfin[i] = jnp.broadcast_to(jnp.max(mx[i], axis=0, keepdims=True), (8, T))

        def pv(n):
            i, j = tiles[n]
            m = mfin[i]
            if hist:
                m = jnp.where(hist[-1] < 0, hist[-1], m)
            p3 = jnp.exp2(sval.pop((i, j)).reshape(T // 8, 8, T) - m[None])
            l8 = jnp.sum(p3, axis=0)
            lsum[i] = l8 if j == 0 else lsum[i] + l8
            hist.append(lsum[i])
            o = _dot(_up(vt_ref[j]), p3.reshape(T, T).astype(BF))
            oacc[i] = o if j == 0 else oacc[i] + o
            if j == i:
                l = jnp.sum(lsum[i], axis=0, keepdims=True)
                ctx_ref[i * HT:(i + 1) * HT, :] = _pk((oacc[i] * (1.0 / l)).T)

        return qk, pv

    def out_proj(h, lo, hi):
        oo = _dot(_up(ctx_ref[lo // 2:hi // 2, :]), _up(wo_ref[h & 1]))
        return [oo[:, t * T:(t + 1) * T] for t in range(NM)]

    def head(after_pv=None):
        qk, pv = attention()
        for t in range(NTL + LAG):
            if t % VI == 0 and t // VI < NS:
                proj_v(t // VI)
            if t < NTL:
                qk(t)
            if t >= LAG:
                pv(t - LAG)
                if after_pv:
                    after_pv(t - LAG)

    def prep(h):
        prep_k(h)
        prep_q(h)
        prep_v(h)

    z = jnp.int32(0)
    wk0, wv0, wq0 = w_copies(z)
    x_copy(0).start()
    for cp in [wk0, wv0, wq0] + c_copies(0):
        cp.start()
    for r in range(1, NR):
        for cp in c_copies(r) + [x_copy(r)]:
            cp.start()
    y_ref[...] = jnp.zeros(y_ref.shape, F32)
    wr = jnp.broadcast_to(wr_ref[...].reshape(1, M), (NS, M))
    sub = lax.broadcasted_iota(I32, (NS, T), 0)
    score = [jnp.zeros((NS, T), F32)]
    G = R // T

    def route(s):
        xx = jnp.concatenate([_up(xn_ref[t, s * HT:(s + 1) * HT, :]) for t in range(NM)], axis=1)
        score[0] = jnp.where(sub == s, _dot_nt(wr, xx), score[0])

    qk, pv = attention()
    x_copy(0).wait()
    for s in range(G):
        layernorm(s)
    for cp in [wk0, wv0, wq0] + c_copies(0):
        cp.wait()
    prep(z)
    proj_k(0)
    proj_q(0)
    for s in range(G):
        proj_v(s)
        route(s)
    nq = npv = 0
    for r in range(1, NR):
        for cp in c_copies(r) + [x_copy(r)]:
            cp.wait()
        if r == 1:
            for cp in [wo_copy(z)] + w_copies(z + 1):
                cp.start()
        if r == 2:
            for cp in [wo_copy(z + 1)] + f_copies(z + 1) + f_copies(z + 2):
                cp.start()
        if r == NR - 1:
            for cp in [wo_copy(z)] + w_copies(z + 1):
                cp.wait()
        proj_k(r)
        q_to = min(first(r * G), nq + Q0)
        p_to = max(first((r - 1) * G), q_to - LAG) if r < NR - 1 else q_to - LAG
        q0, p0 = nq, npv
        for u in range(G):
            layernorm(r * G + u)
            proj_v(r * G + u)
            qe, pe = q0 + (q_to - q0) * (u + 1) // G, p0 + (p_to - p0) * (u + 1) // G
            while nq < qe or npv < pe:
                if nq < qe:
                    qk(nq)
                    nq += 1
                if npv < pe:
                    pv(npv)
                    npv += 1
        proj_q(r)
        for u in range(G):
            route(r * G + u)

    score = _rb(score[0])
    row8 = lax.broadcasted_iota(I32, (CAP, T), 0)
    st = dict(key=jnp.where(score != score, -jnp.inf, score), pos=sub * T + lax.broadcasted_iota(I32, (NS, T), 1),
              gate=jnp.zeros((CAP, T), F32), xs=[jnp.zeros((CAP, T), F32) for _ in range(NM)])

    def pick(i):
        key, pos = st["key"], st["pos"]
        best = jnp.max(jnp.max(key, axis=0, keepdims=True), axis=1, keepdims=True)
        cand = jnp.where(key == best, pos, S)
        sel = jnp.min(jnp.min(cand, axis=0, keepdims=True), axis=1, keepdims=True)
        hit = pos == sel
        st["key"] = jnp.where(hit, -jnp.inf, key)
        st["pos"] = jnp.where(hit, S, pos)
        st["gate"] = jnp.where(row8 == i, best, st["gate"])
        tok = jnp.minimum(sel[0, 0], S - 1)
        idx_ref[i] = tok
        for t in range(NM):
            st["xs"][t] = jnp.where(row8 == i, _half(xn_ref[t, pl.ds(tok >> 1, 1), :], tok & 1), st["xs"][t])

    npick = 0
    while npv < NTL:
        if nq < NTL:
            qk(nq)
            nq += 1
        if nq - npv >= LAG or nq == NTL:
            pv(npv)
            npv += 1
            if npv % 8 == 0 and npick < CAP:
                pick(npick)
                npick += 1
    assert npick == CAP
    xs_ref[...] = jnp.concatenate(st["xs"], axis=1)
    gate = _rb(1.0 / (1.0 + jnp.exp(-st["gate"])))
    prep(z + 1)
    for r in range(NR):
        oo = out_proj(0, r * R, (r + 1) * R)
        for t in range(NM):
            acc_ref[t, r * R:(r + 1) * R, :] = oo[t]
    wo_copy(z + 2).start()
    for cp in w_copies(z + 2) + w_copies(z + 3):
        cp.start()

    def body(h, carry):
        for cp in [wo_copy(h)] + f_copies(h) + w_copies(h + 1):
            cp.wait()
        xsel = xs_ref[...].astype(BF)
        proj_k(0)
        g = _rb(_dot_nt(xsel, _up(ffn_ref[h & 1, 0])))
        proj_k(1)
        u = _rb(_dot_nt(xsel, _up(ffn_ref[h & 1, 1])))
        proj_k(2)
        proj_k(3)
        hcol = f_start(h) + lax.broadcasted_iota(I32, (CAP, T), 1)
        hid = jnp.where(hcol >= (h - 1) * T, _rb(g / (1.0 + jnp.exp(-g))) * u, 0.0).astype(BF)
        proj_q(0)
        y_ref[...] += _dot(hid, _up(ffn_ref[h & 1, 2]))
        for r in range(1, NR):
            proj_q(r)
        head()
        prep(h + 1)
        for r in range(NR):
            oo = out_proj(h, r * R, (r + 1) * R)
            for t in range(NM):
                acc_ref[t, r * R:(r + 1) * R, :] += oo[t]
        for cp in [wo_copy(h + 2)] + f_copies(h + 2) + w_copies(h + 3):
            cp.start()
        return carry

    lax.fori_loop(1, H - 1, body, 0)

    wo_copy(z + H - 1).wait()
    y = _rb(_rb(y_ref[...]) * gate[:, :1])
    for i in range(CAP):
        tok = idx_ref[i]
        for t in range(NM):
            acc_ref[t, pl.ds(tok, 1), :] += y[i:i + 1, t * T:(t + 1) * T]
    for r in range(NR):
        proj_k(r)
        proj_q(r)
        rows = slice(r * R, (r + 1) * R)
        for t in range(NM):
            acc_ref[t, rows, :] += x_ref[rows, t * T:(t + 1) * T].astype(F32) + _up(xn_ref[t, r * HR:(r + 1) * HR, :]).astype(F32)

    def finish(lo, hi):
        oo = out_proj(H - 1, lo, hi)
        for t in range(NM):
            x_ref[lo:hi, t * T:(t + 1) * T] = (acc_ref[t, lo:hi, :] + oo[t]).astype(BF)

    outs = [o_copy(k, CUTS[k], CUTS[k + 1]) for k in range(len(CUTS) - 1)]
    plan = {}
    for lo in range(0, CUTS[-2], FC):
        hi = min(lo + FC, min(c for c in CUTS if c > lo))
        at = min(first(hi // T) + 8, NTL - 1)
        plan.setdefault(at, []).append(functools.partial(finish, lo, hi))
        if hi in CUTS:
            plan.setdefault(min(at + 6, NTL - 1), []).append(outs[CUTS.index(hi) - 1].start)
    head(lambda n: [fn() for fn in plan.get(n, ())])
    finish(CUTS[-2], S)
    outs[-1].start()
    for cp in [wo_copy(z + H)] + f_copies(z + H - 1) + f_copies(z + H) + w_copies(z + H) + w_copies(z + H + 1):
        cp.wait()
    for cp in outs:
        cp.wait()

@jax.jit
def pallas_parallel_sum__compressed_kv_cla__moe_arch_mod__prompt_kernel(
    A_x, A_c_kv, A_w_q, A_w_uk, A_w_uv, A_w_o, B_x, B_w_r, B_w_gate, B_w_up, B_w_down):
    B, S, M = A_x.shape
    Dc = A_c_kv.shape[2]
    H, D = A_w_q.shape[1:]
    FD = B_w_gate.shape[1]
    NP = H // 2
    hbm = pl.BlockSpec(memory_space=pltpu.HBM)
    dma = pltpu.SemaphoreType.DMA
    out = pl.pallas_call(
        functools.partial(kernel, S=S, M=M, D=D, H=H, FD=FD),
        in_specs=[hbm] * 6 + [pl.BlockSpec(memory_space=pltpu.VMEM)] + [hbm] * 3,
        out_specs=hbm,
        out_shape=jax.ShapeDtypeStruct((B, S, M), BF),
        scratch_shapes=[
            pltpu.VMEM((S, M), BF),
            pltpu.VMEM((M // T, S // 2, T), U32), pltpu.VMEM((S // 2, Dc), U32), pltpu.VMEM((M // T, S, T), F32),
            pltpu.VMEM((S // 2, D), U32), pltpu.VMEM((S // 2, D), U32), pltpu.VMEM((S // T, D // 2, T), U32),
            pltpu.VMEM((S // 2, D), U32),
            pltpu.VMEM((2, M, D), U32), pltpu.VMEM((2, Dc, D), U32), pltpu.VMEM((2, Dc, D), U32), pltpu.VMEM((2, D // 2, M), U32),
            pltpu.VMEM((M // 2, D), U32), pltpu.VMEM((Dc // 2, D), U32), pltpu.VMEM((D // 2, Dc), U32),
            pltpu.VMEM((2, 3, HT, M), U32), pltpu.VMEM((CAP, M), F32), pltpu.VMEM((CAP, M), F32), pltpu.SMEM((CAP,), I32),
            dma((6,)), dma((2,)), dma((6,)), dma((S // R,)), dma((S // R,)),
        ],
        compiler_params=pltpu.CompilerParams(vmem_limit_bytes=120 * 2**20, disable_bounds_checks=NB),
    )(A_x, A_c_kv, A_w_q.reshape(M, NP, 2, D), A_w_uk.reshape(Dc, NP, 2, D), A_w_uv.reshape(Dc, NP, 2, D),
      A_w_o, B_w_r, B_w_gate.T, B_w_up.T, B_w_down)
    return out
```

```python
import functools, math
import jax
import jax.numpy as jnp
from jax import lax
import jax.experimental.pallas as pl
import jax.experimental.pallas.tpu as pltpu

BF = jnp.bfloat16
F32 = jnp.float32
U32 = jnp.uint32
I32 = jnp.int32
NT = (((1,), (1,)), ((), ()))
T = 128
HT = T // 2
R = 512
HR = R // 2
LAG = 40
VI = 2
CAP = 8
FS = 85
F0 = 58
Q0 = 6
FC = 256
CUTS = [0,1280,1792,2048]
NB = True
PIN = 1

def _dot(a, b):
    return jnp.dot(a, b, preferred_element_type=F32)

def _dot_nt(a, b):
    return lax.dot_general(a, b, NT, preferred_element_type=F32)

def _pk(x):
    return pltpu.bitcast(x.astype(BF), U32)

def _up(x):
    return pltpu.bitcast(x, BF)

def _rb(x):
    return x.astype(BF).astype(F32)

def _half(w32, odd):
    sh = ((1 - odd) * 16).astype(U32)
    return pltpu.bitcast((w32 << sh) & jnp.uint32(0xFFFF0000), F32)

def kernel(x_hbm, c_hbm, wq_hbm, wk_hbm, wv_hbm, wo_hbm, wr_ref, wg_hbm, wu_hbm, wd_hbm, o_hbm,
           x_ref, xn_ref, cs_ref, acc_ref, q_ref, k_ref, vt_ref, ctx_ref,
           rq_ref, rk_ref, rv_ref, wo_ref, wq_ref, wk_ref, wvt_ref, ffn_ref, xs_ref, idx_ref,
           s_w, s_f, s_x, s_c, *, S, M, D, H, FD):
    scale = (D ** -0.5) * math.log2(math.e)
    NM = M // T
    NS = S // T
    NR = S // R

    def w_copies(p):
        cps = [pltpu.make_async_copy(w.bitcast(U32).at[:, p, 0, :], b.at[p], s_w.at[p * 4 + i])
               for i, (w, b) in enumerate(((wk_hbm, rk_ref), (wv_hbm, rv_ref), (wq_hbm, rq_ref)))]
        return cps + [pltpu.make_async_copy(wo_hbm.bitcast(U32).at[p], wo_ref.at[p], s_w.at[p * 4 + 3])]

    f_copies = [pltpu.make_async_copy(w.bitcast(U32), ffn_ref.at[i], s_f.at[i])
                for i, w in enumerate((wg_hbm, wu_hbm, wd_hbm))]

    def x_copy(r):
        return pltpu.make_async_copy(x_hbm.at[0, r * R:(r + 1) * R, :], x_ref.at[r * R:(r + 1) * R, :], s_x.at[r])

    def c_copies(r):
        rs = slice(r * HR, (r + 1) * HR)
        return [pltpu.make_async_copy(c_hbm.bitcast(U32).at[0, rs, :], cs_ref.at[rs, :], s_c.at[r])]

    def o_copy(k, lo, hi):
        return pltpu.make_async_copy(x_ref.at[lo:hi, :], o_hbm.at[0, lo:hi, :], s_x.at[k])

    def prep_k(h):
        wk_ref[...] = _pk(_half(rk_ref[h >> 1], h & 1))

    def prep_q(h):
        wq_ref[...] = _pk(_half(rq_ref[h >> 1], h & 1))

    def prep_v(h):
        wvt_ref[...] = _pk(_half(rv_ref[h >> 1], h & 1).T)

    def proj_k(r):
        rs = slice(r * HR, (r + 1) * HR)
        cc = _up(cs_ref[rs, :])
        k_ref[rs, :] = _pk(_dot(cc, _up(wk_ref[...])))

    def proj_q(r):
        rs = slice(r * HR, (r + 1) * HR)
        xx = jnp.concatenate([_up(xn_ref[t, rs, :]) for t in range(NM)], axis=1)
        q_ref[rs, :] = _pk(_dot(xx, _up(wq_ref[...])) * scale)

    def proj_v(s):
        rs = slice(s * HT, (s + 1) * HT)
        cc = _up(cs_ref[rs, :])
        vt_ref[s] = _pk(_dot_nt(_up(wvt_ref[...]), cc))

    def layernorm(s):
        x = x_ref[s * T:(s + 1) * T, :].astype(F32)
        m = jnp.sum(x, axis=-1, keepdims=True) * (1.0 / M)
        mb = _rb(m)
        d = x - mb
        v = jnp.sum(d * d, axis=-1, keepdims=True) * (1.0 / M) - (m - mb) * (m - mb)
        den = _rb(jnp.sqrt(_rb(_rb(v) + 1e-5)))
        xn = (d * (1.0 / den)).astype(BF)
        for t in range(NM):
            xn_ref[t, s * HT:(s + 1) * HT, :] = pltpu.bitcast(xn[:, t * T:(t + 1) * T], U32)
        return xn

    tiles = [(i, j) for i in range(NS) for j in range(i + 1)]
    NTL = len(tiles)

    def first(i):
        return i * (i + 1) // 2

    def attention():
        key = lax.broadcasted_iota(I32, (T, T), 0)
        qry = lax.broadcasted_iota(I32, (T, T), 1)
        tri = key <= qry
        sval, mx, mfin, lsum, oacc, hist = {}, {}, {}, {}, {}, []

        def qk(n):
            i, j = tiles[n]
            s = _dot_nt(_up(k_ref[j * HT:(j + 1) * HT, :]), _up(q_ref[i * HT:(i + 1) * HT, :]))
            if j == i:
                s = jnp.where(tri, s, -1e9)
            sval[i, j] = s
            m8 = jnp.max(s.reshape(T // 8, 8, T), axis=0)
            mx[i] = m8 if j == 0 else jnp.maximum(mx[i], m8)
            if j == i:
                mfin[i] = jnp.broadcast_to(jnp.max(mx[i], axis=0, keepdims=True), (8, T))

        def pv(n):
            i, j = tiles[n]
            m = mfin[i]
            if hist:
                m = jnp.where(hist[-1] < 0, hist[-1], m)
            p3 = jnp.exp2(sval.pop((i, j)).reshape(T // 8, 8, T) - m[None])
            l8 = jnp.sum(p3, axis=0)
            lsum[i] = l8 if j == 0 else lsum[i] + l8
            hist.append(lsum[i])
            o = _dot(_up(vt_ref[j]), p3.reshape(T, T).astype(BF))
            oacc[i] = o if j == 0 else oacc[i] + o
            if j == i:
                l = jnp.sum(lsum[i], axis=0, keepdims=True)
                ctx_ref[i * HT:(i + 1) * HT, :] = _pk((oacc[i] * (1.0 / l)).T)

        return qk, pv

    def out_proj(h, lo, hi):
        oo = _dot(_up(ctx_ref[lo // 2:hi // 2, :]), _up(wo_ref[h >> 1, pl.ds(pl.multiple_of((h & 1) * HT, HT), HT), :]))
        return [oo[:, t * T:(t + 1) * T] for t in range(NM)]

    def head(after_pv=None, at_t=None):
        qk, pv = attention()
        for t in range(NTL + LAG):
            if t % VI == 0 and t // VI < NS:
                proj_v(t // VI)
            if at_t:
                at_t(t)
            if t < NTL:
                qk(t)
            if t >= LAG:
                pv(t - LAG)
                if after_pv:
                    after_pv(t - LAG)

    def prep(h):
        prep_k(h)
        prep_q(h)
        prep_v(h)

    z = jnp.int32(0)
    w0 = w_copies(0)
    (c0,), (c1,), (c2,), (c3,) = [c_copies(r) for r in range(NR)]
    x0, x1, x2, x3 = [x_copy(r) for r in range(NR)]
    for cp in [x0, x1] + w0[:3] + [c0, x2, c1, x3, c2, c3]:
        cp.start()
    wr = jnp.broadcast_to(wr_ref[...].reshape(1, M), (NS, M))
    sub = lax.broadcasted_iota(I32, (NS, T), 0)
    score = [jnp.zeros((NS, T), F32)]
    G = R // T

    def route(s):
        xx = jnp.concatenate([_up(xn_ref[t, s * HT:(s + 1) * HT, :]) for t in range(NM)], axis=1)
        score[0] = jnp.where(sub == s, _dot_nt(wr, xx), score[0])

    qk, pv = attention()
    cur = [0, 0]

    def advance(q_to, p_to):
        while cur[0] < q_to or cur[1] < p_to:
            if cur[0] < q_to:
                qk(cur[0])
                cur[0] += 1
            if cur[1] < p_to:
                pv(cur[1])
                cur[1] += 1

    x0.wait()
    for s in range(G):
        layernorm(s)
    x1.wait()
    for s in range(G, 2 * G):
        layernorm(s)
    for cp in w0[:3] + [c0]:
        cp.wait()
    prep(z)
    proj_k(0)
    proj_q(0)
    proj_q(1)
    for s in range(G):
        proj_v(s)
        route(s)
        route(G + s)
        advance(first(s + 1), 0)
    x2.wait()
    c1.wait()
    for cp in w0[3:] + w_copies(1):
        cp.start()
    proj_k(1)
    for u in range(G):
        layernorm(2 * G + u)
        proj_v(G + u)
        advance(first(G + u + 1), first(u + 1))
    proj_q(2)
    for cp in [x3, c2, c3, w0[3]]:
        cp.wait()
    proj_k(2)
    layernorm(3 * G)
    proj_v(2 * G)
    proj_v(2 * G + 1)
    layernorm(3 * G + 1)
    proj_k(3)
    layernorm(3 * G + 2)
    proj_v(2 * G + 2)
    proj_v(2 * G + 3)
    layernorm(3 * G + 3)
    for u in range(G):
        proj_v(3 * G + u)
        route(2 * G + u)
        advance(cur[0] + Q0, cur[1] + Q0 // 2)
    proj_q(3)
    for u in range(G):
        route(3 * G + u)

    score = _rb(score[0])
    row8 = lax.broadcasted_iota(I32, (CAP, T), 0)
    st = dict(key=jnp.where(score != score, -jnp.inf, score), pos=sub * T + lax.broadcasted_iota(I32, (NS, T), 1),
              gate=jnp.zeros((CAP, T), F32), xs=[jnp.zeros((CAP, T), F32) for _ in range(NM)])

    def pick(i):
        key, pos = st["key"], st["pos"]
        best = jnp.max(jnp.max(key, axis=0, keepdims=True), axis=1, keepdims=True)
        cand = jnp.where(key == best, pos, S)
        sel = jnp.min(jnp.min(cand, axis=0, keepdims=True), axis=1, keepdims=True)
        hit = pos == sel
        st["key"] = jnp.where(hit, -jnp.inf, key)
        st["pos"] = jnp.where(hit, S, pos)
        st["gate"] = jnp.where(row8 == i, best, st["gate"])
        tok = jnp.minimum(sel[0, 0], S - 1)
        idx_ref[i] = tok
        for t in range(NM):
            st["xs"][t] = jnp.where(row8 == i, _half(xn_ref[t, pl.ds(tok >> 1, 1), :], tok & 1), st["xs"][t])

    npick = 0
    while cur[1] < NTL:
        lagged = cur[0] - cur[1] >= LAG or cur[0] == NTL
        advance(min(cur[0] + 1, NTL), cur[1] + lagged)
        if lagged and cur[1] % 8 == 0 and npick < CAP:
            pick(npick)
            npick += 1
    assert npick == CAP
    xs_ref[...] = jnp.concatenate(st["xs"], axis=1)
    gate = _rb(1.0 / (1.0 + jnp.exp(-st["gate"])))
    prep(z + 1)
    for r in range(NR):
        oo = out_proj(z, r * R, (r + 1) * R)
        for t in range(NM):
            base = (x_ref[r * R:(r + 1) * R, t * T:(t + 1) * T].astype(F32)
                    + _up(xn_ref[t, r * HR:(r + 1) * HR, :]).astype(F32))
            acc_ref[t, r * R:(r + 1) * R, :] = base + oo[t]
    for cp in f_copies:
        cp.start()

    def body(h, carry):
        def next_pair(_, c):
            p = (h + 1) >> 1
            for cp in w_copies(p):
                cp.wait()

            @pl.when(p + 1 < H // 2)
            def _():
                for cp in w_copies(p + 1):
                    cp.start()
            return c

        lax.fori_loop(0, h & 1, next_pair, 0)
        for r in range(NR):
            proj_k(r)
        for r in range(NR):
            proj_q(r)
        head()
        prep(h + 1)
        for r in range(NR):
            oo = out_proj(h, r * R, (r + 1) * R)
            for t in range(NM):
                acc_ref[t, r * R:(r + 1) * R, :] += oo[t]
        return carry

    lax.fori_loop(1, H - 1, body, 0)

    for cp in f_copies:
        cp.wait()
    chunks = [(lo, min(lo + T, FD)) for lo in range(0, FD, T)]
    part, hid = {}, {}

    def ffn_in(k, w, t):
        lo, hi = chunks[k]
        d = _dot_nt(xs_ref[:, t * T:(t + 1) * T].astype(BF), _up(ffn_ref[w, lo // 2:hi // 2, t * T:(t + 1) * T]))
        part[k, w] = d if t == 0 else part[k, w] + d
        if w == 1 and t == NM - 1:
            g = _rb(part[k, 0])
            hid[k] = (_rb(g / (1.0 + jnp.exp(-g))) * _rb(part[k, 1])).astype(BF)

    def ffn_out(k, t):
        lo, hi = chunks[k]
        d = _dot(hid[k], _up(ffn_ref[2, lo // 2:hi // 2, t * T:(t + 1) * T]))
        part[t] = d if k == 0 else part[t] + d

    def ffn_scatter():
        for t in range(NM):
            y = _rb(_rb(part[t]) * gate)
            for i in range(CAP):
                acc_ref[t, pl.ds(idx_ref[i], 1), :] += y[i:i + 1, :]

    todo = [functools.partial(ffn_in, k, w, t) for k in range(len(chunks)) for w in range(2) for t in range(NM)]
    todo += [functools.partial(ffn_out, k, t) for k in range(len(chunks)) for t in range(NM)]
    todo += [None] * (-len(todo) % 4 + 8) + [ffn_scatter]

    def ffn_step():
        for fn in todo[:4]:
            if fn:
                fn()
        del todo[:4]

    for r in range(NR):
        proj_k(r)
        ffn_step()
        proj_q(r)
        ffn_step()

    def finish(lo, hi):
        assert not todo
        oo = out_proj(z + H - 1, lo, hi)
        for t in range(NM):
            x_ref[lo:hi, t * T:(t + 1) * T] = (acc_ref[t, lo:hi, :] + oo[t]).astype(BF)

    outs = [o_copy(k, CUTS[k], CUTS[k + 1]) for k in range(len(CUTS) - 1)]
    plan = {}
    for lo in range(0, CUTS[-2], FC):
        hi = min(lo + FC, min(c for c in CUTS if c > lo))
        at = min(max(first(hi // T) + 8, F0 + lo // FS), NTL - 1)
        plan.setdefault(at, []).append(functools.partial(finish, lo, hi))
        if hi in CUTS:
            plan.setdefault(min(at + 6, NTL - 1), []).append(outs[CUTS.index(hi) - 1].start)
    head(lambda n: [fn() for fn in plan.get(n, ())], lambda t: ffn_step() if t % 2 == 1 else None)
    assert not todo
    finish(CUTS[-2], S)
    outs[-1].start()
    for cp in outs:
        cp.wait()

@jax.jit
def pallas_parallel_sum__compressed_kv_cla__moe_arch_mod__prompt_kernel(
    A_x, A_c_kv, A_w_q, A_w_uk, A_w_uv, A_w_o, B_x, B_w_r, B_w_gate, B_w_up, B_w_down):
    B, S, M = A_x.shape
    Dc = A_c_kv.shape[2]
    H, D = A_w_q.shape[1:]
    FD = B_w_gate.shape[1]
    NP = H // 2
    hbm = pl.BlockSpec(memory_space=pltpu.HBM)
    dma = pltpu.SemaphoreType.DMA
    out = pl.pallas_call(
        functools.partial(kernel, S=S, M=M, D=D, H=H, FD=FD),
        in_specs=[hbm] * 6 + [pl.BlockSpec(memory_space=pltpu.VMEM)] + [hbm] * 3,
        out_specs=hbm,
        out_shape=jax.ShapeDtypeStruct((B, S, M), BF),
        scratch_shapes=[
            pltpu.VMEM((S, M), BF),
            pltpu.VMEM((M // T, S // 2, T), U32), pltpu.VMEM((S // 2, Dc), U32), pltpu.VMEM((M // T, S, T), F32),
            pltpu.VMEM((S // 2, D), U32), pltpu.VMEM((S // 2, D), U32), pltpu.VMEM((S // T, D // 2, T), U32),
            pltpu.VMEM((S // 2, D), U32),
            pltpu.VMEM((NP, M, D), U32), pltpu.VMEM((NP, Dc, D), U32), pltpu.VMEM((NP, Dc, D), U32), pltpu.VMEM((NP, D, M), U32),
            pltpu.VMEM((M // 2, D), U32), pltpu.VMEM((Dc // 2, D), U32), pltpu.VMEM((D // 2, Dc), U32),
            pltpu.VMEM((3, FD // 2, M), U32), pltpu.VMEM((CAP, M), F32), pltpu.SMEM((CAP,), I32),
            dma((4 * NP,)), dma((3,)), dma((S // R,)), dma((S // R,)),
        ],
        compiler_params=pltpu.CompilerParams(vmem_limit_bytes=120 * 2**20, disable_bounds_checks=NB),
    )(A_x, A_c_kv, A_w_q.reshape(M, NP, 2, D), A_w_uk.reshape(Dc, NP, 2, D), A_w_uv.reshape(Dc, NP, 2, D),
      A_w_o.reshape(NP, 2 * D, M), B_w_r, B_w_gate.T, B_w_up.T, B_w_down)
    return out
```

```python
import functools, math
import jax
import jax.numpy as jnp
from jax import lax
import jax.experimental.pallas as pl
import jax.experimental.pallas.tpu as pltpu

BF = jnp.bfloat16
F32 = jnp.float32
U32 = jnp.uint32
I32 = jnp.int32
NT = (((1,), (1,)), ((), ()))
T = 128
HT = T // 2
R = 512
HR = R // 2
LAG = 42
VI = 2
LR = 16
CAP = 8
CUTS = [0, 1280, 1792, 2048]
FC, F0, FS = 128, 58, 85


def _dot(a, b):
    return jnp.dot(a, b, preferred_element_type=F32)

def _dot_nt(a, b):
    return lax.dot_general(a, b, NT, preferred_element_type=F32)

def _pk(x):
    return pltpu.bitcast(x.astype(BF), U32)

def _up(x):
    return pltpu.bitcast(x, BF)

def _rb(x):
    return x.astype(BF).astype(F32)

def _half(w32, odd):
    sh = ((1 - odd) * 16).astype(U32)
    return pltpu.bitcast((w32 << sh) & jnp.uint32(0xFFFF0000), F32)

def kernel(x_hbm, c_hbm, wq_hbm, wk_hbm, wv_hbm, wo_hbm, wr_ref, wg_hbm, wu_hbm, wd_hbm, o_hbm,
           x_ref, xn_ref, cs_ref, acc_ref, q_ref, k_ref, vt_ref, ctx_ref,
           rq_ref, rk_ref, rv_ref, wo_ref, wq_ref, wk_ref, wvt_ref, ffn_ref, xs_ref, idx_ref,
           s_w, s_f, s_x, s_c, *, S, M, D, H, FD):
    scale = (D ** -0.5) * math.log2(math.e)
    NM = M // T
    NS = S // T
    NR = S // R

    def w_copies(p):
        cps = [pltpu.make_async_copy(w.bitcast(U32).at[:, p, 0, :], b.at[p], s_w.at[p * 4 + i])
               for i, (w, b) in enumerate(((wk_hbm, rk_ref), (wv_hbm, rv_ref), (wq_hbm, rq_ref)))]
        return cps + [pltpu.make_async_copy(wo_hbm.bitcast(U32).at[p], wo_ref.at[p], s_w.at[p * 4 + 3])]

    f_copies = [pltpu.make_async_copy(w.bitcast(U32), ffn_ref.at[i], s_f.at[i])
                for i, w in enumerate((wg_hbm, wu_hbm, wd_hbm))]

    def x_copy(r):
        return pltpu.make_async_copy(x_hbm.at[0, r * R:(r + 1) * R, :], x_ref.at[r * R:(r + 1) * R, :], s_x.at[r])

    def c_copies(r):
        rs = slice(r * HR, (r + 1) * HR)
        return [pltpu.make_async_copy(c_hbm.bitcast(U32).at[0, rs, :], cs_ref.at[rs, :], s_c.at[r])]

    def o_copy(k, lo, hi):
        return pltpu.make_async_copy(x_ref.at[lo:hi, :], o_hbm.at[0, lo:hi, :], s_x.at[k])

    def prep_k(h):
        wk_ref[...] = _pk(_half(rk_ref[h >> 1], h & 1))

    def prep_q(h):
        wq_ref[...] = _pk(_half(rq_ref[h >> 1], h & 1))

    def prep_v(h):
        wvt_ref[...] = _pk(_half(rv_ref[h >> 1], h & 1).T)

    def proj_k(r):
        rs = slice(r * HR, (r + 1) * HR)
        cc = _up(cs_ref[rs, :])
        k_ref[rs, :] = _pk(_dot(cc, _up(wk_ref[...])))

    def proj_q(r, hr=HR):
        rs = slice(r * hr, (r + 1) * hr)
        xx = jnp.concatenate([_up(xn_ref[t, rs, :]) for t in range(NM)], axis=1)
        q_ref[rs, :] = _pk(_dot(xx, _up(wq_ref[...])) * scale)

    def proj_v(s):
        rs = slice(s * HT, (s + 1) * HT)
        cc = _up(cs_ref[rs, :])
        vt_ref[s] = _pk(_dot_nt(_up(wvt_ref[...]), cc))

    def layernorm(s):
        x = x_ref[s * LR:(s + 1) * LR, :].astype(F32)
        m = jnp.sum(x, axis=-1, keepdims=True) * (1.0 / M)
        mb = _rb(m)
        d = x - mb
        v = jnp.sum(d * d, axis=-1, keepdims=True) * (1.0 / M) - (m - mb) * (m - mb)
        v = jnp.maximum(v, 0.0)
        den = _rb(jnp.sqrt(_rb(_rb(v) + 1e-5)))
        xn = (d * (1.0 / den)).astype(BF)
        for t in range(NM):
            xn_ref[t, s * LR // 2:(s + 1) * LR // 2, :] = pltpu.bitcast(xn[:, t * T:(t + 1) * T], U32)
        return xn

    tiles = [(i, j) for i in range(NS) for j in range(i + 1)]
    NTL = len(tiles)

    def first(i):
        return i * (i + 1) // 2

    def attention():
        key = lax.broadcasted_iota(I32, (T, T), 0)
        qry = lax.broadcasted_iota(I32, (T, T), 1)
        tri = key <= qry
        sval, mx, mfin, lsum, oacc, hist = {}, {}, {}, {}, {}, []
        after = {}

        def qk(n):
            i, j = tiles[n]
            s = _dot_nt(_up(k_ref[j * HT:(j + 1) * HT, :]), _up(q_ref[i * HT:(i + 1) * HT, :]))
            if j == i:
                s = jnp.where(tri, s, -1e9 * math.log2(math.e))
            sval[i, j] = s
            m8 = jnp.max(s.reshape(T // 8, 8, T), axis=0)
            mx[i] = m8 if j == 0 else jnp.maximum(mx[i], m8)
            if j == i:
                mfin[i] = jnp.broadcast_to(jnp.max(mx[i], axis=0, keepdims=True), (8, T))

        def pv(n):
            i, j = tiles[n]
            m = mfin[i]
            if hist:
                m = jnp.where(hist[-1] < 0, hist[-1], m)
            if n in after:
                m = jnp.where(after[n] < 0, 0.0, m)
            p3 = jnp.exp2(sval.pop((i, j)).reshape(T // 8, 8, T) - m[None])
            l8 = jnp.sum(p3, axis=0)
            lsum[i] = l8 if j == 0 else lsum[i] + l8
            hist.append(lsum[i])
            o = _dot(_up(vt_ref[j]), p3.reshape(T, T).astype(BF))
            oacc[i] = o if j == 0 else oacc[i] + o
            if j == i:
                l = jnp.sum(lsum[i], axis=0, keepdims=True)
                ctx_ref[i * HT:(i + 1) * HT, :] = _pk((oacc[i] * (1.0 / l)).T)

        return qk, pv, after

    def out_proj(h, lo, hi):
        oo = _dot(_up(ctx_ref[lo // 2:hi // 2, :]), _up(wo_ref[h >> 1, pl.ds(pl.multiple_of((h & 1) * HT, HT), HT), :]))
        return [oo[:, t * T:(t + 1) * T] for t in range(NM)]

    def head(after_pv=None, at_t=None):
        qk, pv, _ = attention()
        for t in range(NTL + LAG):
            if t % VI == 0 and t // VI < NS:
                proj_v(t // VI)
            if at_t:
                at_t(t)
            if t < NTL:
                qk(t)
            if t >= LAG:
                pv(t - LAG)
                if after_pv:
                    after_pv(t - LAG)

    def prep(h):
        prep_k(h)
        prep_q(h)
        prep_v(h)

    z = jnp.int32(0)
    w0 = w_copies(0)
    (c0,), (c1,), (c2,), (c3,) = [c_copies(r) for r in range(NR)]
    x0, x1, x2, x3 = [x_copy(r) for r in range(NR)]
    for cp in [x0, w0[2], x1, x2, x3, w0[0], w0[1], c0, c1, c2, c3]:
        cp.start()
    wr = jnp.broadcast_to(wr_ref[...].reshape(1, M), (NS, M))
    sub = lax.broadcasted_iota(I32, (NS, T), 0)
    score = [jnp.zeros((NS, T), F32)]
    G = R // T

    def route(s):
        xx = jnp.concatenate([_up(xn_ref[t, s * HT:(s + 1) * HT, :]) for t in range(NM)], axis=1)
        score[0] = jnp.where(sub == s, _dot_nt(wr, xx), score[0])

    qk, pv, after = attention()
    cur = [0, 0]

    def advance(q_to, p_to):
        while cur[0] < q_to or cur[1] < p_to:
            if cur[0] < q_to:
                qk(cur[0])
                cur[0] += 1
            if cur[1] < p_to:
                pv(cur[1])
                cur[1] += 1

    for r, cps in enumerate(([x0], [w0[2], x1], [x2], [x3])):
        for cp in cps:
            cp.wait()
        if r == 1:
            prep_q(z)
        for u in range(G):
            for w in range(T // LR):
                layernorm((r * G + u) * (T // LR) + w)
                if r > 0 and w == 0:
                    proj_q((r - 1) * G + u, HT)
            if r > 0:
                route((r - 1) * G + u)
    for cp in [w0[0], w0[1], c0]:
        cp.wait()
    prep_k(z)
    prep_v(z)
    proj_q(NR - 1)
    proj_k(0)
    for s in range(G):
        route((NR - 1) * G + s)
        proj_v(s)
        advance(first(s + 1), 0)
    c1.wait()
    c2.wait()
    for cp in w0[3:] + w_copies(1):
        cp.start()
    proj_k(1)
    proj_k(2)
    for s in range(G, 2 * G):
        proj_v(s)
        advance(first(s + 1), max(first(s - G + 1), first(s + 1) - 20))
    for cp in [c3, w0[3]]:
        cp.wait()
    proj_k(3)
    for s in range(2 * G, NS):
        proj_v(s)
        advance(cur[0] + 3, cur[1])

    score = _rb(score[0])
    row8 = lax.broadcasted_iota(I32, (CAP, T), 0)
    st = dict(key=jnp.where(score != score, -jnp.inf, score), pos=sub * T + lax.broadcasted_iota(I32, (NS, T), 1),
              gate=jnp.zeros((CAP, T), F32), xs=[jnp.zeros((CAP, T), F32) for _ in range(NM)])

    def pick(i):
        key, pos = st["key"], st["pos"]
        best = jnp.max(jnp.max(key, axis=0, keepdims=True), axis=1, keepdims=True)
        cand = jnp.where(key == best, pos, S)
        sel = jnp.min(jnp.min(cand, axis=0, keepdims=True), axis=1, keepdims=True)
        hit = pos == sel
        st["key"] = jnp.where(hit, -jnp.inf, key)
        st["pos"] = jnp.where(hit, S, pos)
        st["gate"] = jnp.where(row8 == i, best, st["gate"])
        tok = jnp.minimum(sel[0, 0], S - 1)
        idx_ref[i] = tok
        after[cur[1] + 7] = sel
        for t in range(NM):
            st["xs"][t] = jnp.where(row8 == i, _half(xn_ref[t, pl.ds(tok >> 1, 1), :], tok & 1), st["xs"][t])

    npick = 0
    while cur[1] < NTL:
        lagged = cur[0] - cur[1] >= LAG or cur[0] == NTL
        advance(min(cur[0] + 1, NTL), cur[1] + lagged)
        if lagged and cur[1] % 8 == 0 and npick < CAP:
            pick(npick)
            npick += 1
    assert npick == CAP
    xs_ref[...] = jnp.concatenate(st["xs"], axis=1)
    gate = _rb(1.0 / (1.0 + jnp.exp(-st["gate"])))
    prep(z + 1)
    for r in range(NR):
        oo = out_proj(z, r * R, (r + 1) * R)
        for t in range(NM):
            base = (x_ref[r * R:(r + 1) * R, t * T:(t + 1) * T].astype(F32)
                    + _up(xn_ref[t, r * HR:(r + 1) * HR, :]).astype(F32))
            acc_ref[t, r * R:(r + 1) * R, :] = base + oo[t]
    for cp in f_copies:
        cp.start()

    def body(h, carry):
        def next_pair(_, c):
            p = (h + 1) >> 1
            for cp in w_copies(p):
                cp.wait()

            @pl.when(p + 1 < H // 2)
            def _():
                for cp in w_copies(p + 1):
                    cp.start()
            return c

        lax.fori_loop(0, h & 1, next_pair, 0)
        for r in range(NR):
            proj_k(r)
        for r in range(NR):
            proj_q(r)
        head()
        prep(h + 1)
        for r in range(NR):
            oo = out_proj(h, r * R, (r + 1) * R)
            for t in range(NM):
                acc_ref[t, r * R:(r + 1) * R, :] += oo[t]
        return carry

    lax.fori_loop(1, H - 1, body, 0)

    for cp in f_copies:
        cp.wait()
    chunks = [(lo, min(lo + T, FD)) for lo in range(0, FD, T)]
    part, hid = {}, {}

    def ffn_in(k, w, t):
        lo, hi = chunks[k]
        d = _dot_nt(xs_ref[:, t * T:(t + 1) * T].astype(BF), _up(ffn_ref[w, lo // 2:hi // 2, t * T:(t + 1) * T]))
        part[k, w] = d if t == 0 else part[k, w] + d
        if w == 1 and t == NM - 1:
            g = _rb(part[k, 0])
            hid[k] = (_rb(g / (1.0 + jnp.exp(-g))) * _rb(part[k, 1])).astype(BF)

    def ffn_out(k, t):
        lo, hi = chunks[k]
        d = _dot(hid[k], _up(ffn_ref[2, lo // 2:hi // 2, t * T:(t + 1) * T]))
        part[t] = d if k == 0 else part[t] + d

    def ffn_scatter():
        for t in range(NM):
            y = _rb(_rb(part[t]) * gate)
            for i in range(CAP):
                acc_ref[t, pl.ds(idx_ref[i], 1), :] += y[i:i + 1, :]

    todo = [functools.partial(ffn_in, k, w, t) for k in range(len(chunks)) for w in range(2) for t in range(NM)]
    todo += [functools.partial(ffn_out, k, t) for k in range(len(chunks)) for t in range(NM)]
    todo += [None] * (-len(todo) % 4 + 8) + [ffn_scatter]

    def ffn_step():
        for fn in todo[:4]:
            if fn:
                fn()
        del todo[:4]

    for r in range(NR):
        proj_k(r)
        ffn_step()
        proj_q(r)
        ffn_step()

    def finish(lo, hi):
        assert not todo
        oo = out_proj(z + H - 1, lo, hi)
        for t in range(NM):
            x_ref[lo:hi, t * T:(t + 1) * T] = (acc_ref[t, lo:hi, :] + oo[t]).astype(BF)

    outs = [o_copy(k, CUTS[k], CUTS[k + 1]) for k in range(len(CUTS) - 1)]
    plan = {}
    for lo in range(0, CUTS[-2], FC):
        hi = min(lo + FC, min(c for c in CUTS if c > lo))
        at = min(max(first(hi // T) + 8, F0 + lo // FS), NTL - 1)
        plan.setdefault(at, []).append(functools.partial(finish, lo, hi))
        if hi in CUTS:
            plan.setdefault(min(at + 6, NTL - 1), []).append(outs[CUTS.index(hi) - 1].start)
    head(lambda n: [fn() for fn in plan.get(n, ())], lambda t: ffn_step() if t % 2 == 1 else None)
    assert not todo
    finish(CUTS[-2], S)
    outs[-1].start()
    for cp in outs:
        cp.wait()

@jax.jit
def pallas_parallel_sum__compressed_kv_cla__moe_arch_mod__prompt_kernel(
    A_x, A_c_kv, A_w_q, A_w_uk, A_w_uv, A_w_o, B_x, B_w_r, B_w_gate, B_w_up, B_w_down):
    B, S, M = A_x.shape
    Dc = A_c_kv.shape[2]
    H, D = A_w_q.shape[1:]
    FD = B_w_gate.shape[1]
    NP = H // 2
    hbm = pl.BlockSpec(memory_space=pltpu.HBM)
    dma = pltpu.SemaphoreType.DMA
    out = pl.pallas_call(
        functools.partial(kernel, S=S, M=M, D=D, H=H, FD=FD),
        in_specs=[hbm] * 6 + [pl.BlockSpec(memory_space=pltpu.VMEM)] + [hbm] * 3,
        out_specs=hbm,
        out_shape=jax.ShapeDtypeStruct((B, S, M), BF),
        scratch_shapes=[
            pltpu.VMEM((S, M), BF),
            pltpu.VMEM((M // T, S // 2, T), U32), pltpu.VMEM((S // 2, Dc), U32), pltpu.VMEM((M // T, S, T), F32),
            pltpu.VMEM((S // 2, D), U32), pltpu.VMEM((S // 2, D), U32), pltpu.VMEM((S // T, D // 2, T), U32),
            pltpu.VMEM((S // 2, D), U32),
            pltpu.VMEM((NP, M, D), U32), pltpu.VMEM((NP, Dc, D), U32), pltpu.VMEM((NP, Dc, D), U32), pltpu.VMEM((NP, D, M), U32),
            pltpu.VMEM((M // 2, D), U32), pltpu.VMEM((Dc // 2, D), U32), pltpu.VMEM((D // 2, Dc), U32),
            pltpu.VMEM((3, FD // 2, M), U32), pltpu.VMEM((CAP, M), F32), pltpu.SMEM((CAP,), I32),
            dma((4 * NP,)), dma((3,)), dma((S // R,)), dma((S // R,)),
        ],
        compiler_params=pltpu.CompilerParams(vmem_limit_bytes=120 * 2**20),
    )(A_x, A_c_kv, A_w_q.reshape(M, NP, 2, D), A_w_uk.reshape(Dc, NP, 2, D), A_w_uv.reshape(Dc, NP, 2, D),
      A_w_o.reshape(NP, 2 * D, M), B_w_r, B_w_gate.T, B_w_up.T, B_w_down)
    return out
```

```python
import functools, math
import jax
import jax.numpy as jnp
from jax import lax
import jax.experimental.pallas as pl
import jax.experimental.pallas.tpu as pltpu

BF = jnp.bfloat16
F32 = jnp.float32
U32 = jnp.uint32
I32 = jnp.int32
NT = (((1,), (1,)), ((), ()))
T = 128
HT = T // 2
R = 512
HR = R // 2
LAG = 42
VI = 3
CAP = 8
AH = 19
LR = 16
FS = 85
F0 = 58
FC = 128
CUTS = [0,1280,1792,2048]

def _dot(a, b):
    return jnp.dot(a, b, preferred_element_type=F32)

def _dot_nt(a, b):
    return lax.dot_general(a, b, NT, preferred_element_type=F32)

def _pk(x):
    return pltpu.bitcast(x.astype(BF), U32)

def _up(x):
    return pltpu.bitcast(x, BF)

def _rb(x):
    return x.astype(BF).astype(F32)

def _half(w32, odd):
    sh = ((1 - odd) * 16).astype(U32)
    return pltpu.bitcast((w32 << sh) & jnp.uint32(0xFFFF0000), F32)

def kernel(x_hbm, c_hbm, wq_hbm, wk_hbm, wv_hbm, wo_hbm, wr_ref, wg_hbm, wu_hbm, wd_hbm, o_hbm,
           x_ref, xn_ref, cs_ref, acc_ref, q_ref, k_ref, vt_ref, ctx_ref,
           rq_ref, rk_ref, rv_ref, bq_ref, bk_ref, bv_ref, wo_ref, wq_ref, wk_ref, wvt_ref, ffn_ref, xs_ref, idx_ref,
           s_w, s_f, s_x, s_c, *, S, M, D, H, FD):
    scale = (D ** -0.5) * math.log2(math.e)
    NM = M // T
    NS = S // T
    NR = S // R

    w_hbm = (wk_hbm, wv_hbm, wq_hbm)
    w0 = [pltpu.make_async_copy(w.bitcast(U32).at[:, 0, 0, :], b, s_w.at[i])
          for i, (w, b) in enumerate(zip(w_hbm, (rk_ref, rv_ref, rq_ref)))]
    w0.append(pltpu.make_async_copy(wo_hbm.bitcast(U32).at[0:1], wo_ref.at[0:1], s_w.at[3]))
    wo_rest = pltpu.make_async_copy(wo_hbm.bitcast(U32).at[1:], wo_ref.at[1:], s_w.at[4])

    def w_group(g):
        return [pltpu.make_async_copy(w.bitcast(U32).at[:, g * 8:(g + 1) * 8, 0, :],
                                      b.at[g * (w.shape[0] + 1):g * (w.shape[0] + 1) + w.shape[0]], s_w.at[5 + g * 3 + i])
                for i, (w, b) in enumerate(zip(w_hbm, (bk_ref, bv_ref, bq_ref)))]

    def raw(small, big, h):
        if isinstance(h, int):
            return _half(small[...], jnp.int32(h))
        n = small.shape[0]
        flat = big.reshape(big.shape[0] * 8, D)
        return _half(flat[pl.ds((h >> 4) * (n + 1) * 8 + ((h >> 1) & 7), n, stride=8), :], h & 1)

    f_copies = [pltpu.make_async_copy(w.bitcast(U32), ffn_ref.at[i], s_f.at[i])
                for i, w in enumerate((wg_hbm, wu_hbm, wd_hbm))]

    def x_copy(r):
        return pltpu.make_async_copy(x_hbm.at[0, r * R:(r + 1) * R, :], x_ref.at[r * R:(r + 1) * R, :], s_x.at[r])

    def c_copies(r):
        rs = slice(r * HR, (r + 1) * HR)
        return [pltpu.make_async_copy(c_hbm.bitcast(U32).at[0, rs, :], cs_ref.at[rs, :], s_c.at[r])]

    def o_copy(k, lo, hi):
        return pltpu.make_async_copy(x_ref.at[lo:hi, :], o_hbm.at[0, lo:hi, :], s_x.at[k])

    def prep_k(h):
        wk_ref[...] = _pk(raw(rk_ref, bk_ref, h))

    def prep_q(h):
        wq_ref[...] = _pk(raw(rq_ref, bq_ref, h))

    def prep_v(h):
        wvt_ref[...] = _pk(raw(rv_ref, bv_ref, h).T)

    def proj_k(r):
        rs = slice(r * HR, (r + 1) * HR)
        cc = _up(cs_ref[rs, :])
        k_ref[rs, :] = _pk(_dot(cc, _up(wk_ref[...])))

    def proj_q(r, hr=HR):
        rs = slice(r * hr, (r + 1) * hr)
        xx = jnp.concatenate([_up(xn_ref[t, rs, :]) for t in range(NM)], axis=1)
        q_ref[rs, :] = _pk(_dot(xx, _up(wq_ref[...])) * scale)

    def proj_v(s):
        rs = slice(s * HT, (s + 1) * HT)
        cc = _up(cs_ref[rs, :])
        vt_ref[s] = _pk(_dot_nt(_up(wvt_ref[...]), cc))

    def layernorm(s):
        x = x_ref[s * LR:(s + 1) * LR, :].astype(F32)
        m = jnp.sum(x, axis=-1, keepdims=True) * (1.0 / M)
        mb = _rb(m)
        d = x - mb
        v = jnp.sum(d * d, axis=-1, keepdims=True) * (1.0 / M) - (m - mb) * (m - mb)
        v = jnp.maximum(v, 0.0)
        den = _rb(jnp.sqrt(_rb(_rb(v) + 1e-5)))
        xn = (d * (1.0 / den)).astype(BF)
        for t in range(NM):
            xn_ref[t, s * LR // 2:(s + 1) * LR // 2, :] = pltpu.bitcast(xn[:, t * T:(t + 1) * T], U32)
        return xn

    tiles = [(i, j) for i in range(NS) for j in range(i + 1)]
    NTL = len(tiles)

    def first(i):
        return i * (i + 1) // 2

    def attention():
        key = lax.broadcasted_iota(I32, (T, T), 0)
        qry = lax.broadcasted_iota(I32, (T, T), 1)
        tri = key <= qry
        sval, mx, mfin, lsum, oacc, hist = {}, {}, {}, {}, {}, []
        after, seen = {}, []

        def qk(n):
            i, j = tiles[n]
            s = _dot_nt(_up(k_ref[j * HT:(j + 1) * HT, :]), _up(q_ref[i * HT:(i + 1) * HT, :]))
            if j == i:
                s = jnp.where(tri, s, -1e9 * math.log2(math.e))
            sval[i, j] = s
            m8 = jnp.max(s.reshape(T // 8, 8, T), axis=0)
            seen.append(m8)
            mx[i] = m8 if j == 0 else jnp.maximum(mx[i], m8)
            if j == i:
                mfin[i] = jnp.broadcast_to(jnp.max(mx[i], axis=0, keepdims=True), (8, T))

        def pv(n):
            i, j = tiles[n]
            m = mfin[i]
            if hist:
                dep = hist[-1]
                if AH > 0 and n + AH < NTL and len(seen) > n + AH + 4:
                    dep = jnp.maximum(dep, seen[n + AH])
                m = jnp.where(dep < 0, dep, m)
            if n in after:
                m = jnp.where(after[n] < 0, 0.0, m)
            p3 = jnp.exp2(sval.pop((i, j)).reshape(T // 8, 8, T) - m[None])
            l8 = jnp.sum(p3, axis=0)
            lsum[i] = l8 if j == 0 else lsum[i] + l8
            hist.append(lsum[i])
            o = _dot(_up(vt_ref[j]), p3.reshape(T, T).astype(BF))
            oacc[i] = o if j == 0 else oacc[i] + o
            if j == i:
                l = jnp.sum(lsum[i], axis=0, keepdims=True)
                ctx_ref[i * HT:(i + 1) * HT, :] = _pk((oacc[i] * (1.0 / l)).T)

        return qk, pv, after

    def out_proj(h, lo, hi):
        oo = _dot(_up(ctx_ref[lo // 2:hi // 2, :]), _up(wo_ref[h >> 1, pl.ds(pl.multiple_of((h & 1) * HT, HT), HT), :]))
        return [oo[:, t * T:(t + 1) * T] for t in range(NM)]

    def head(after_pv=None, at_t=None):
        qk, pv, _ = attention()
        for t in range(NTL + LAG):
            if t % VI == 0 and t // VI < NS:
                proj_v(t // VI)
            if at_t:
                at_t(t)
            if t < NTL:
                qk(t)
            if t >= LAG:
                pv(t - LAG)
                if after_pv:
                    after_pv(t - LAG)

    def prep(h):
        prep_k(h)
        prep_q(h)
        prep_v(h)

    z = jnp.int32(0)
    (c0,), (c1,), (c2,), (c3,) = [c_copies(r) for r in range(NR)]
    x0, x1, x2, x3 = [x_copy(r) for r in range(NR)]
    for cp in [x0, w0[2], x1, x2, x3, w0[0], w0[1], c0, c1, c2, c3]:
        cp.start()
    wr = jnp.broadcast_to(wr_ref[...].reshape(1, M), (NS, M))
    sub = lax.broadcasted_iota(I32, (NS, T), 0)
    score = [jnp.zeros((NS, T), F32)]
    G = R // T

    def route(s):
        xx = jnp.concatenate([_up(xn_ref[t, s * HT:(s + 1) * HT, :]) for t in range(NM)], axis=1)
        score[0] = jnp.where(sub == s, _dot_nt(wr, xx), score[0])

    qk, pv, after = attention()
    cur = [0, 0]

    def advance(q_to, p_to):
        while cur[0] < q_to or cur[1] < p_to:
            if cur[0] < q_to:
                qk(cur[0])
                cur[0] += 1
            if cur[1] < p_to:
                pv(cur[1])
                cur[1] += 1

    for r, cps in enumerate(([x0], [w0[2], x1], [x2], [x3])):
        for cp in cps:
            cp.wait()
        if r == 1:
            prep_q(0)
        for u in range(G):
            for w in range(T // LR):
                layernorm((r * G + u) * (T // LR) + w)
                if r > 0 and w == 0:
                    proj_q((r - 1) * G + u, HT)
            if r > 0:
                route((r - 1) * G + u)
    for cp in [w0[0], w0[1], c0]:
        cp.wait()
    prep_k(0)
    prep_v(0)
    proj_q(NR - 1)
    proj_k(0)
    for s in range(G):
        route((NR - 1) * G + s)
        proj_v(s)
        advance(first(s + 1), 0)
    c1.wait()
    c2.wait()
    for cp in [w0[3]] + w_group(0):
        cp.start()
    proj_k(1)
    proj_k(2)
    for s in range(G, 2 * G):
        proj_v(s)
        advance(first(s + 1), max(first(s - G + 1), first(s + 1) - 20))
    for cp in [c3, w0[3]]:
        cp.wait()
    proj_k(3)
    for s in range(2 * G, NS):
        proj_v(s)
        advance(cur[0] + 3, cur[1])

    score = _rb(score[0])
    row8 = lax.broadcasted_iota(I32, (CAP, T), 0)
    st = dict(key=jnp.where(score != score, -jnp.inf, score), pos=sub * T + lax.broadcasted_iota(I32, (NS, T), 1),
              gate=jnp.zeros((CAP, T), F32), xs=[jnp.zeros((CAP, T), F32) for _ in range(NM)])

    def pick(i):
        key, pos = st["key"], st["pos"]
        best = jnp.max(jnp.max(key, axis=0, keepdims=True), axis=1, keepdims=True)
        cand = jnp.where(key == best, pos, S)
        sel = jnp.min(jnp.min(cand, axis=0, keepdims=True), axis=1, keepdims=True)
        hit = pos == sel
        st["key"] = jnp.where(hit, -jnp.inf, key)
        st["pos"] = jnp.where(hit, S, pos)
        st["gate"] = jnp.where(row8 == i, best, st["gate"])
        tok = jnp.minimum(sel[0, 0], S - 1)
        idx_ref[i] = tok
        after[cur[1] + 7] = sel
        for t in range(NM):
            st["xs"][t] = jnp.where(row8 == i, _half(xn_ref[t, pl.ds(tok >> 1, 1), :], tok & 1), st["xs"][t])

    npick = 0
    while cur[1] < NTL:
        lagged = cur[0] - cur[1] >= LAG or cur[0] == NTL
        advance(min(cur[0] + 1, NTL), cur[1] + lagged)
        if lagged and cur[1] % 8 == 0 and npick < CAP:
            pick(npick)
            npick += 1
    assert npick == CAP
    xs_ref[...] = jnp.concatenate(st["xs"], axis=1)
    gate = _rb(1.0 / (1.0 + jnp.exp(-st["gate"])))
    prep(1)
    for r in range(NR):
        oo = out_proj(z, r * R, (r + 1) * R)
        for t in range(NM):
            base = (x_ref[r * R:(r + 1) * R, t * T:(t + 1) * T].astype(F32)
                    + _up(xn_ref[t, r * HR:(r + 1) * HR, :]).astype(F32))
            acc_ref[t, r * R:(r + 1) * R, :] = base + oo[t]
    for cp in [wo_rest] + w_group(1) + f_copies:
        cp.start()
    for cp in w_group(0):
        cp.wait()

    def body(h, carry):
        pl.when(h == 2)(wo_rest.wait)

        @pl.when(h == 8)
        def _():
            for cp in w_group(1):
                cp.wait()

        for r in range(NR):
            proj_k(r)
        for r in range(NR):
            proj_q(r)
        head()
        prep(h + 1)
        for r in range(NR):
            oo = out_proj(h, r * R, (r + 1) * R)
            for t in range(NM):
                acc_ref[t, r * R:(r + 1) * R, :] += oo[t]
        return carry

    lax.fori_loop(1, H - 1, body, 0)

    for cp in f_copies:
        cp.wait()
    chunks = [(lo, min(lo + T, FD)) for lo in range(0, FD, T)]
    part, hid = {}, {}

    def ffn_in(k, w, t):
        lo, hi = chunks[k]
        d = _dot_nt(xs_ref[:, t * T:(t + 1) * T].astype(BF), _up(ffn_ref[w, lo // 2:hi // 2, t * T:(t + 1) * T]))
        part[k, w] = d if t == 0 else part[k, w] + d
        if w == 1 and t == NM - 1:
            g = _rb(part[k, 0])
            hid[k] = (_rb(g / (1.0 + jnp.exp(-g))) * _rb(part[k, 1])).astype(BF)

    def ffn_out(k, t):
        lo, hi = chunks[k]
        d = _dot(hid[k], _up(ffn_ref[2, lo // 2:hi // 2, t * T:(t + 1) * T]))
        part[t] = d if k == 0 else part[t] + d

    def ffn_scatter():
        for t in range(NM):
            y = _rb(_rb(part[t]) * gate)
            for i in range(CAP):
                acc_ref[t, pl.ds(idx_ref[i], 1), :] += y[i:i + 1, :]

    todo = [functools.partial(ffn_in, k, w, t) for k in range(len(chunks)) for w in range(2) for t in range(NM)]
    todo += [functools.partial(ffn_out, k, t) for k in range(len(chunks)) for t in range(NM)]
    todo += [None] * (-len(todo) % 4 + 8) + [ffn_scatter]

    def ffn_step():
        for fn in todo[:4]:
            if fn:
                fn()
        del todo[:4]

    for r in range(NR):
        proj_k(r)
        ffn_step()
        proj_q(r)
        ffn_step()

    def finish(lo, hi):
        assert not todo
        oo = out_proj(z + H - 1, lo, hi)
        for t in range(NM):
            x_ref[lo:hi, t * T:(t + 1) * T] = (acc_ref[t, lo:hi, :] + oo[t]).astype(BF)

    outs = [o_copy(k, CUTS[k], CUTS[k + 1]) for k in range(len(CUTS) - 1)]
    plan = {}
    for lo in range(0, CUTS[-2], FC):
        hi = min(lo + FC, min(c for c in CUTS if c > lo))
        at = min(max(first(hi // T) + 8, F0 + lo // FS), NTL - 1)
        plan.setdefault(at, []).append(functools.partial(finish, lo, hi))
        if hi in CUTS:
            plan.setdefault(min(at + 6, NTL - 1), []).append(outs[CUTS.index(hi) - 1].start)
    head(lambda n: [fn() for fn in plan.get(n, ())], lambda t: ffn_step() if t % 2 == 1 else None)
    assert not todo
    finish(CUTS[-2], S)
    outs[-1].start()
    for cp in outs:
        cp.wait()

@jax.jit
def pallas_parallel_sum__compressed_kv_cla__moe_arch_mod__prompt_kernel(
    A_x, A_c_kv, A_w_q, A_w_uk, A_w_uv, A_w_o, B_x, B_w_r, B_w_gate, B_w_up, B_w_down):
    B, S, M = A_x.shape
    Dc = A_c_kv.shape[2]
    H, D = A_w_q.shape[1:]
    FD = B_w_gate.shape[1]
    NP = H // 2
    hbm = pl.BlockSpec(memory_space=pltpu.HBM)
    dma = pltpu.SemaphoreType.DMA
    out = pl.pallas_call(
        functools.partial(kernel, S=S, M=M, D=D, H=H, FD=FD),
        in_specs=[hbm] * 6 + [pl.BlockSpec(memory_space=pltpu.VMEM)] + [hbm] * 3,
        out_specs=hbm,
        out_shape=jax.ShapeDtypeStruct((B, S, M), BF),
        scratch_shapes=[
            pltpu.VMEM((S, M), BF),
            pltpu.VMEM((M // T, S // 2, T), U32), pltpu.VMEM((S // 2, Dc), U32), pltpu.VMEM((M // T, S, T), F32),
            pltpu.VMEM((S // 2, D), U32), pltpu.VMEM((S // 2, D), U32), pltpu.VMEM((S // T, D // 2, T), U32),
            pltpu.VMEM((S // 2, D), U32),
            pltpu.VMEM((M, D), U32), pltpu.VMEM((Dc, D), U32), pltpu.VMEM((Dc, D), U32),
            pltpu.VMEM((2 * (M + 1), 8, D), U32), pltpu.VMEM((2 * (Dc + 1), 8, D), U32), pltpu.VMEM((2 * (Dc + 1), 8, D), U32),
            pltpu.VMEM((NP, D, M), U32),
            pltpu.VMEM((M // 2, D), U32), pltpu.VMEM((Dc // 2, D), U32), pltpu.VMEM((D // 2, Dc), U32),
            pltpu.VMEM((3, FD // 2, M), U32), pltpu.VMEM((CAP, M), F32), pltpu.SMEM((CAP,), I32),
            dma((11,)), dma((3,)), dma((S // R,)), dma((S // R,)),
        ],
        compiler_params=pltpu.CompilerParams(vmem_limit_bytes=120 * 2**20),
    )(A_x, A_c_kv, A_w_q.reshape(M, NP, 2, D), A_w_uk.reshape(Dc, NP, 2, D), A_w_uv.reshape(Dc, NP, 2, D),
      A_w_o.reshape(NP, 2 * D, M), B_w_r, B_w_gate.T, B_w_up.T, B_w_down)
    return out
```

```python
import functools, math
import jax
import jax.numpy as jnp
from jax import lax
import jax.experimental.pallas as pl
import jax.experimental.pallas.tpu as pltpu

BF = jnp.bfloat16
F32 = jnp.float32
U32 = jnp.uint32
I32 = jnp.int32
NT = (((1,), (1,)), ((), ()))
T = 128
HT = T // 2
R = 512
HR = R // 2
LAG = 42
VI = 3
CAP = 8
SP = 4
FP = 3
AH = 19
LR = 16
FS = 85
F0 = 30
FC = 128
CUTS = [0,1280,1664,2048]

def _dot(a, b):
    return jnp.dot(a, b, preferred_element_type=F32)

def _dot_nt(a, b):
    return lax.dot_general(a, b, NT, preferred_element_type=F32)

def _pk(x):
    return pltpu.bitcast(x.astype(BF), U32)

def _up(x):
    return pltpu.bitcast(x, BF)

def _rb(x):
    return x.astype(BF).astype(F32)

def _half(w32, odd):
    sh = ((1 - odd) * 16).astype(U32)
    return pltpu.bitcast((w32 << sh) & jnp.uint32(0xFFFF0000), F32)

def kernel(x_hbm, c_hbm, wq_hbm, wk_hbm, wv_hbm, wo_hbm, wr_ref, wg_hbm, wu_hbm, wd_hbm, o_hbm,
           x_ref, xn_ref, cs_ref, acc_ref, q_ref, k_ref, vt_ref, ctx_ref,
           rq_ref, rk_ref, rv_ref, bq_ref, bk_ref, bv_ref, wo_ref, wq_ref, wk_ref, wvt_ref, ffn_ref, xs_ref, idx_ref,
           s_w, s_f, s_x, s_c, *, S, M, D, H, FD):
    scale = (D ** -0.5) * math.log2(math.e)
    NM = M // T
    NS = S // T
    NR = S // R

    w_hbm = (wk_hbm, wv_hbm, wq_hbm)
    w0 = [pltpu.make_async_copy(w.bitcast(U32).at[:, 0, 0, :], b, s_w.at[i])
          for i, (w, b) in enumerate(zip(w_hbm, (rk_ref, rv_ref, rq_ref)))]
    w0.append(pltpu.make_async_copy(wo_hbm.bitcast(U32).at[0:1], wo_ref.at[0:1], s_w.at[3]))
    wo_rest = pltpu.make_async_copy(wo_hbm.bitcast(U32).at[1:], wo_ref.at[1:], s_w.at[4])

    def w_group(g):
        return [pltpu.make_async_copy(w.bitcast(U32).at[:, g * 8:(g + 1) * 8, 0, :],
                                      b.at[g * (w.shape[0] + 1):g * (w.shape[0] + 1) + w.shape[0]], s_w.at[5 + g * 3 + i])
                for i, (w, b) in enumerate(zip(w_hbm, (bk_ref, bv_ref, bq_ref)))]

    def raw(small, big, h):
        if isinstance(h, int):
            return _half(small[...], jnp.int32(h))
        n = small.shape[0]
        flat = big.reshape(big.shape[0] * 8, D)
        return _half(flat[pl.ds((h >> 4) * (n + 1) * 8 + ((h >> 1) & 7), n, stride=8), :], h & 1)

    f_copies = [pltpu.make_async_copy(w.bitcast(U32), ffn_ref.at[i], s_f.at[i])
                for i, w in enumerate((wg_hbm, wu_hbm, wd_hbm))]

    def x_copy(r):
        return pltpu.make_async_copy(x_hbm.at[0, r * R:(r + 1) * R, :], x_ref.at[r * R:(r + 1) * R, :], s_x.at[r])

    def c_copies(r):
        rs = slice(r * HR, (r + 1) * HR)
        return [pltpu.make_async_copy(c_hbm.bitcast(U32).at[0, rs, :], cs_ref.at[rs, :], s_c.at[r])]

    def o_copy(k, lo, hi):
        return pltpu.make_async_copy(x_ref.at[lo:hi, :], o_hbm.at[0, lo:hi, :], s_x.at[k])

    def prep_k(h):
        wk_ref[...] = _pk(raw(rk_ref, bk_ref, h))

    def prep_q(h):
        wq_ref[...] = _pk(raw(rq_ref, bq_ref, h))

    def prep_v(h):
        wvt_ref[...] = _pk(raw(rv_ref, bv_ref, h).T)

    def proj_k(r, hr=HR):
        rs = slice(r * hr, (r + 1) * hr)
        cc = _up(cs_ref[rs, :])
        k_ref[rs, :] = _pk(_dot(cc, _up(wk_ref[...])))

    def proj_q(r, hr=HR):
        rs = slice(r * hr, (r + 1) * hr)
        xx = jnp.concatenate([_up(xn_ref[t, rs, :]) for t in range(NM)], axis=1)
        q_ref[rs, :] = _pk(_dot(xx, _up(wq_ref[...])) * scale)

    def proj_v(s):
        rs = slice(s * HT, (s + 1) * HT)
        cc = _up(cs_ref[rs, :])
        vt_ref[s] = _pk(_dot_nt(_up(wvt_ref[...]), cc))

    def layernorm(s):
        x = x_ref[s * LR:(s + 1) * LR, :].astype(F32)
        m = jnp.sum(x, axis=-1, keepdims=True) * (1.0 / M)
        mb = _rb(m)
        d = x - mb
        v = jnp.sum(d * d, axis=-1, keepdims=True) * (1.0 / M) - (m - mb) * (m - mb)
        v = jnp.maximum(v, 0.0)
        den = _rb(jnp.sqrt(_rb(_rb(v) + 1e-5)))
        xn = (_rb(d) * (1.0 / den)).astype(BF)
        for t in range(NM):
            xn_ref[t, s * LR // 2:(s + 1) * LR // 2, :] = pltpu.bitcast(xn[:, t * T:(t + 1) * T], U32)
        return xn

    tiles = [(i, j) for i in range(NS) for j in range(i + 1)]
    NTL = len(tiles)

    def first(i):
        return i * (i + 1) // 2

    def attention():
        key = lax.broadcasted_iota(I32, (T, T), 0)
        qry = lax.broadcasted_iota(I32, (T, T), 1)
        tri = key <= qry
        sval, mx, mfin, lsum, oacc, hist = {}, {}, {}, {}, {}, []
        after, seen = {}, []

        def qk(n):
            i, j = tiles[n]
            s = _dot_nt(_up(k_ref[j * HT:(j + 1) * HT, :]), _up(q_ref[i * HT:(i + 1) * HT, :]))
            if j == i:
                s = jnp.where(tri, s, -1e9 * math.log2(math.e))
            sval[i, j] = s
            m8 = jnp.max(s.reshape(T // 8, 8, T), axis=0)
            seen.append(m8)
            mx[i] = m8 if j == 0 else jnp.maximum(mx[i], m8)
            if j == i:
                mfin[i] = jnp.broadcast_to(jnp.max(mx[i], axis=0, keepdims=True), (8, T))

        def pv(n):
            i, j = tiles[n]
            m = mfin[i]
            if hist:
                dep = hist[-1]
                if AH > 0 and n + AH < NTL and len(seen) > n + AH + 4:
                    dep = jnp.maximum(dep, seen[n + AH])
                m = jnp.where(dep < 0, dep, m)
            if n in after:
                m = jnp.where(after[n] < 0, 0.0, m)
            p3 = jnp.exp2(sval.pop((i, j)).reshape(T // 8, 8, T) - m[None])
            l8 = jnp.sum(p3, axis=0)
            lsum[i] = l8 if j == 0 else lsum[i] + l8
            hist.append(lsum[i])
            o = _dot(_up(vt_ref[j]), p3.reshape(T, T).astype(BF))
            oacc[i] = o if j == 0 else oacc[i] + o
            if j == i:
                l = jnp.sum(lsum[i], axis=0, keepdims=True)
                ctx_ref[i * HT:(i + 1) * HT, :] = _pk((oacc[i] * (1.0 / l)).T)

        return qk, pv, after

    def out_proj(h, lo, hi):
        oo = _dot(_up(ctx_ref[lo // 2:hi // 2, :]), _up(wo_ref[h >> 1, pl.ds(pl.multiple_of((h & 1) * HT, HT), HT), :]))
        return [oo[:, t * T:(t + 1) * T] for t in range(NM)]

    def head(after_pv=None, at_t=None):
        qk, pv, _ = attention()
        for t in range(NTL + LAG):
            if t % VI == 0 and t // VI < NS:
                proj_v(t // VI)
            if at_t:
                at_t(t)
            if t < NTL:
                qk(t)
            if t >= LAG:
                pv(t - LAG)
                if after_pv:
                    after_pv(t - LAG)

    def prep(h):
        prep_k(h)
        prep_q(h)
        prep_v(h)

    z = jnp.int32(0)
    (c0,), (c1,), (c2,), (c3,) = [c_copies(r) for r in range(NR)]
    x0, x1, x2, x3 = [x_copy(r) for r in range(NR)]
    for cp in [x0, w0[2], x1, x2, x3, w0[0], w0[1], c0, c1, c2, c3]:
        cp.start()
    wr = jnp.broadcast_to(wr_ref[...].reshape(1, M), (NS, M))
    sub = lax.broadcasted_iota(I32, (NS, T), 0)
    score = [jnp.zeros((NS, T), F32)]
    G = R // T

    def route(s):
        xx = jnp.concatenate([_up(xn_ref[t, s * HT:(s + 1) * HT, :]) for t in range(NM)], axis=1)
        score[0] = jnp.where(sub == s, _dot_nt(wr, xx), score[0])

    qk, pv, after = attention()
    cur = [0, 0]

    def advance(q_to, p_to):
        while cur[0] < q_to or cur[1] < p_to:
            if cur[0] < q_to:
                qk(cur[0])
                cur[0] += 1
            if cur[1] < p_to:
                pv(cur[1])
                cur[1] += 1

    for r, cps in enumerate(([x0], [w0[2], x1], [x2], [x3])):
        for cp in cps:
            cp.wait()
        if r == 1:
            prep_q(0)
        for u in range(G):
            for w in range(T // LR):
                layernorm((r * G + u) * (T // LR) + w)
                if r > 0 and w == 0:
                    proj_q((r - 1) * G + u, HT)
            if r > 0:
                route((r - 1) * G + u)
    for cp in [w0[0], w0[1], c0]:
        cp.wait()
    prep_k(0)
    prep_v(0)
    proj_q(NR - 1)
    proj_k(0)
    for s in range(G):
        route((NR - 1) * G + s)
        proj_v(s)
        advance(first(s + 1), 0)
    c1.wait()
    c2.wait()
    for cp in [w0[3]] + w_group(0):
        cp.start()
    proj_k(1)
    proj_k(2)
    for s in range(G, 2 * G):
        proj_v(s)
        advance(first(s + 1), max(first(s - G + 1), first(s + 1) - 20))
    for cp in [c3, w0[3]]:
        cp.wait()
    proj_k(3)
    for s in range(2 * G, NS):
        proj_v(s)
        advance(cur[0] + 3, cur[1])

    score = _rb(score[0])
    row8 = lax.broadcasted_iota(I32, (CAP, T), 0)
    st = dict(key=jnp.where(score != score, -jnp.inf, score), pos=sub * T + lax.broadcasted_iota(I32, (NS, T), 1),
              gate=jnp.zeros((CAP, T), F32), xs=[jnp.zeros((CAP, T), F32) for _ in range(NM)])

    def pick(i):
        key, pos = st["key"], st["pos"]
        best = jnp.max(jnp.max(key, axis=0, keepdims=True), axis=1, keepdims=True)
        cand = jnp.where(key == best, pos, S)
        sel = jnp.min(jnp.min(cand, axis=0, keepdims=True), axis=1, keepdims=True)
        hit = pos == sel
        st["key"] = jnp.where(hit, -jnp.inf, key)
        st["pos"] = jnp.where(hit, S, pos)
        st["gate"] = jnp.where(row8 == i, best, st["gate"])
        tok = jnp.minimum(sel[0, 0], S - 1)
        idx_ref[i] = tok
        after[cur[1] + 7] = sel
        for t in range(NM):
            st["xs"][t] = jnp.where(row8 == i, _half(xn_ref[t, pl.ds(tok >> 1, 1), :], tok & 1), st["xs"][t])

    npick = 0
    while cur[1] < NTL:
        lagged = cur[0] - cur[1] >= LAG or cur[0] == NTL
        advance(min(cur[0] + 1, NTL), cur[1] + lagged)
        if lagged and cur[1] % 8 == 0 and npick < CAP:
            pick(npick)
            npick += 1
    assert npick == CAP
    xs_ref[...] = jnp.concatenate(st["xs"], axis=1)
    gate = _rb(1.0 / (1.0 + jnp.exp(-st["gate"])))
    prep(1)
    for r in range(NR):
        oo = out_proj(z, r * R, (r + 1) * R)
        for t in range(NM):
            base = (x_ref[r * R:(r + 1) * R, t * T:(t + 1) * T].astype(F32)
                    + _up(xn_ref[t, r * HR:(r + 1) * HR, :]).astype(F32))
            acc_ref[t, r * R:(r + 1) * R, :] = base + oo[t]
    for cp in [wo_rest] + w_group(1) + f_copies:
        cp.start()
    for cp in w_group(0):
        cp.wait()

    def body(h, carry):
        pl.when(h == 2)(wo_rest.wait)

        @pl.when(h == 8)
        def _():
            for cp in w_group(1):
                cp.wait()

        for r in range(NR):
            proj_k(r)
        for r in range(NR):
            proj_q(r)
        head()
        prep(h + 1)
        for r in range(NR):
            oo = out_proj(h, r * R, (r + 1) * R)
            for t in range(NM):
                acc_ref[t, r * R:(r + 1) * R, :] += oo[t]
        return carry

    lax.fori_loop(1, H - 1, body, 0)

    for cp in f_copies:
        cp.wait()
    chunks = [(lo, min(lo + T, FD)) for lo in range(0, FD, T)]
    part, hid = {}, {}

    def ffn_in(k, w, t):
        lo, hi = chunks[k]
        d = _dot_nt(xs_ref[:, t * T:(t + 1) * T].astype(BF), _up(ffn_ref[w, lo // 2:hi // 2, t * T:(t + 1) * T]))
        part[k, w] = d if t == 0 else part[k, w] + d
        if w == 1 and t == NM - 1:
            g = _rb(part[k, 0])
            hid[k] = (_rb(g / (1.0 + jnp.exp(-g))) * _rb(part[k, 1])).astype(BF)

    def ffn_out(k, t):
        lo, hi = chunks[k]
        d = _dot(hid[k], _up(ffn_ref[2, lo // 2:hi // 2, t * T:(t + 1) * T]))
        part[t] = d if k == 0 else part[t] + d

    def ffn_scatter():
        for t in range(NM):
            y = _rb(_rb(part[t]) * gate)
            for i in range(CAP):
                acc_ref[t, pl.ds(idx_ref[i], 1), :] += y[i:i + 1, :]

    todo = [functools.partial(ffn_in, k, w, t) for k in range(len(chunks)) for w in range(2) for t in range(NM)]
    todo += [functools.partial(ffn_out, k, t) for k in range(len(chunks)) for t in range(NM)]
    todo += [None] * (-len(todo) % 4 + 8) + [ffn_scatter]

    def ffn_step():
        for fn in todo[:4]:
            if fn:
                fn()
        del todo[:4]

    for r in range(NR * SP):
        proj_k(r, HR // SP)
        ffn_step()
        proj_q(r, HR // SP)
        ffn_step()

    def finish(lo, hi):
        assert not todo
        oo = out_proj(z + H - 1, lo, hi)
        for t in range(NM):
            x_ref[lo:hi, t * T:(t + 1) * T] = (acc_ref[t, lo:hi, :] + oo[t]).astype(BF)

    outs = [o_copy(k, CUTS[k], CUTS[k + 1]) for k in range(len(CUTS) - 1)]
    plan = {}
    for lo in range(0, CUTS[-2], FC):
        hi = min(lo + FC, min(c for c in CUTS if c > lo))
        at = min(max(first(hi // T) + 8, F0 + lo // FS), NTL - 1)
        plan.setdefault(at, []).append(functools.partial(finish, lo, hi))
        if hi in CUTS:
            plan.setdefault(min(at + 6, NTL - 1), []).append(outs[CUTS.index(hi) - 1].start)
    head(lambda n: [fn() for fn in plan.get(n, ())], lambda t: ffn_step() if t % FP == 1 else None)
    assert not todo
    finish(CUTS[-2], S)
    outs[-1].start()
    for cp in outs:
        cp.wait()

@jax.jit
def pallas_parallel_sum__compressed_kv_cla__moe_arch_mod__prompt_kernel(
    A_x, A_c_kv, A_w_q, A_w_uk, A_w_uv, A_w_o, B_x, B_w_r, B_w_gate, B_w_up, B_w_down):
    B, S, M = A_x.shape
    Dc = A_c_kv.shape[2]
    H, D = A_w_q.shape[1:]
    FD = B_w_gate.shape[1]
    NP = H // 2
    hbm = pl.BlockSpec(memory_space=pltpu.HBM)
    dma = pltpu.SemaphoreType.DMA
    out = pl.pallas_call(
        functools.partial(kernel, S=S, M=M, D=D, H=H, FD=FD),
        in_specs=[hbm] * 6 + [pl.BlockSpec(memory_space=pltpu.VMEM)] + [hbm] * 3,
        out_specs=hbm,
        out_shape=jax.ShapeDtypeStruct((B, S, M), BF),
        scratch_shapes=[
            pltpu.VMEM((S, M), BF),
            pltpu.VMEM((M // T, S // 2, T), U32), pltpu.VMEM((S // 2, Dc), U32), pltpu.VMEM((M // T, S, T), F32),
            pltpu.VMEM((S // 2, D), U32), pltpu.VMEM((S // 2, D), U32), pltpu.VMEM((S // T, D // 2, T), U32),
            pltpu.VMEM((S // 2, D), U32),
            pltpu.VMEM((M, D), U32), pltpu.VMEM((Dc, D), U32), pltpu.VMEM((Dc, D), U32),
            pltpu.VMEM((2 * (M + 1), 8, D), U32), pltpu.VMEM((2 * (Dc + 1), 8, D), U32), pltpu.VMEM((2 * (Dc + 1), 8, D), U32),
            pltpu.VMEM((NP, D, M), U32),
            pltpu.VMEM((M // 2, D), U32), pltpu.VMEM((Dc // 2, D), U32), pltpu.VMEM((D // 2, Dc), U32),
            pltpu.VMEM((3, FD // 2, M), U32), pltpu.VMEM((CAP, M), F32), pltpu.SMEM((CAP,), I32),
            dma((11,)), dma((3,)), dma((S // R,)), dma((S // R,)),
        ],
        compiler_params=pltpu.CompilerParams(vmem_limit_bytes=120 * 2**20),
    )(A_x, A_c_kv, A_w_q.reshape(M, NP, 2, D), A_w_uk.reshape(Dc, NP, 2, D), A_w_uv.reshape(Dc, NP, 2, D),
      A_w_o.reshape(NP, 2 * D, M), B_w_r, B_w_gate.T, B_w_up.T, B_w_down)
    return out
```

```python
import functools, math
import numpy as np
import jax
import jax.numpy as jnp
from jax import lax
import jax.experimental.pallas as pl
import jax.experimental.pallas.tpu as pltpu

BF = jnp.bfloat16
F32 = jnp.float32
U32 = jnp.uint32
I32 = jnp.int32
NT = (((1,), (1,)), ((), ()))
T = 128
HT = T // 2
R = 512
HR = R // 2
LAG = 42
VI = 3
CAP = 8
AH = 19
LR = 16
SP, FP = 4, 3
FC, F0, FS = 128, 30, 85
CUTS = [0, 1280, 1664, 2048]


def _dot(a, b):
    return jnp.dot(a, b, preferred_element_type=F32)

def _dot_nt(a, b):
    return lax.dot_general(a, b, NT, preferred_element_type=F32)

def _pk(x):
    return pltpu.bitcast(x.astype(BF), U32)

def _up(x):
    return pltpu.bitcast(x, BF)

def _rb(x):
    return x.astype(BF).astype(F32)

def _half(w32, odd):
    sh = (1 - odd) * 16
    sh = np.uint32(sh) if isinstance(sh, int) else sh.astype(U32)
    return pltpu.bitcast((w32 << sh) & np.uint32(0xFFFF0000), F32)

def kernel(x_hbm, c_hbm, wq_hbm, wk_hbm, wv_hbm, wo_hbm, wr_ref, wg_hbm, wu_hbm, wd_hbm, o_hbm,
           x_ref, xn_ref, cs_ref, acc_ref, q_ref, k_ref, vt_ref, ctx_ref,
           rq_ref, rk_ref, rv_ref, bq_ref, bk_ref, bv_ref, wo_ref, wq_ref, wk_ref, wvt_ref, ffn_ref, xs_ref, idx_ref,
           s_w, s_f, s_x, s_c, *, S, M, D, H, FD):
    scale = (D ** -0.5) * math.log2(math.e)
    NM = M // T
    NS = S // T
    NR = S // R

    w_hbm = (wk_hbm, wv_hbm, wq_hbm)
    w0 = [pltpu.make_async_copy(w.bitcast(U32).at[:, 0, 0, :], b, s_w.at[i])
          for i, (w, b) in enumerate(zip(w_hbm, (rk_ref, rv_ref, rq_ref)))]
    w0.append(pltpu.make_async_copy(wo_hbm.bitcast(U32).at[0:1], wo_ref.at[0:1], s_w.at[3]))
    wo_rest = pltpu.make_async_copy(wo_hbm.bitcast(U32).at[1:], wo_ref.at[1:], s_w.at[4])

    def w_group(g):
        return [pltpu.make_async_copy(w.bitcast(U32).at[:, g * 8:(g + 1) * 8, 0, :],
                                      b.at[g * (w.shape[0] + 1):g * (w.shape[0] + 1) + w.shape[0]], s_w.at[5 + g * 3 + i])
                for i, (w, b) in enumerate(zip(w_hbm, (bk_ref, bv_ref, bq_ref)))]

    def raw(small, big, h):
        if isinstance(h, int):
            return _half(small[...], h)
        n = small.shape[0]
        flat = big.reshape(big.shape[0] * 8, D)
        return _half(flat[pl.ds((h >> 4) * (n + 1) * 8 + ((h >> 1) & 7), n, stride=8), :], h & 1)

    f_copies = [pltpu.make_async_copy(w.bitcast(U32), ffn_ref.at[i], s_f.at[i])
                for i, w in enumerate((wg_hbm, wu_hbm, wd_hbm))]

    def x_copy(r):
        return pltpu.make_async_copy(x_hbm.at[0, r * R:(r + 1) * R, :], x_ref.at[r * R:(r + 1) * R, :], s_x.at[r])

    def c_copies(r):
        rs = slice(r * HR, (r + 1) * HR)
        return [pltpu.make_async_copy(c_hbm.bitcast(U32).at[0, rs, :], cs_ref.at[rs, :], s_c.at[r])]

    def o_copy(k, lo, hi):
        return pltpu.make_async_copy(x_ref.at[lo:hi, :], o_hbm.at[0, lo:hi, :], s_x.at[k])

    def prep_k(h):
        wk_ref[...] = _pk(raw(rk_ref, bk_ref, h))

    def prep_q(h):
        wq_ref[...] = _pk(raw(rq_ref, bq_ref, h))

    def prep_v(h):
        wvt_ref[...] = _pk(raw(rv_ref, bv_ref, h).T)

    def proj_k(r, hr=HR):
        rs = slice(r * hr, (r + 1) * hr)
        cc = _up(cs_ref[rs, :])
        k_ref[rs, :] = _pk(_dot(cc, _up(wk_ref[...])))

    def proj_q(r, hr=HR):
        rs = slice(r * hr, (r + 1) * hr)
        xx = jnp.concatenate([_up(xn_ref[t, rs, :]) for t in range(NM)], axis=1)
        q_ref[rs, :] = _pk(_dot(xx, _up(wq_ref[...])) * scale)

    def proj_v(s):
        rs = slice(s * HT, (s + 1) * HT)
        cc = _up(cs_ref[rs, :])
        vt_ref[s] = _pk(_dot_nt(_up(wvt_ref[...]), cc))

    def layernorm(s):
        x = x_ref[s * LR:(s + 1) * LR, :].astype(F32)
        m = jnp.sum(x, axis=-1, keepdims=True) * (1.0 / M)
        mb = _rb(m)
        d = x - mb
        v = jnp.sum(d * d, axis=-1, keepdims=True) * (1.0 / M) - (m - mb) * (m - mb)
        v = jnp.maximum(v, 0.0)
        den = _rb(jnp.sqrt(_rb(_rb(v) + 1e-5)))
        xn = (_rb(d) * (1.0 / den)).astype(BF)
        for t in range(NM):
            xn_ref[t, s * LR // 2:(s + 1) * LR // 2, :] = pltpu.bitcast(xn[:, t * T:(t + 1) * T], U32)

    tiles = [(i, j) for i in range(NS) for j in range(i + 1)]
    NTL = len(tiles)

    def first(i):
        return i * (i + 1) // 2

    def attention():
        key = lax.broadcasted_iota(I32, (T, T), 0)
        qry = lax.broadcasted_iota(I32, (T, T), 1)
        tri = key <= qry
        sval, mx, mfin, lsum, oacc, hist = {}, {}, {}, {}, {}, []
        after, seen = {}, []

        def qk(n):
            i, j = tiles[n]
            s = _dot_nt(_up(k_ref[j * HT:(j + 1) * HT, :]), _up(q_ref[i * HT:(i + 1) * HT, :]))
            if j == i:
                s = jnp.where(tri, s, -1e9 * math.log2(math.e))
            sval[i, j] = s
            m8 = jnp.max(s.reshape(T // 8, 8, T), axis=0)
            seen.append(m8)
            mx[i] = m8 if j == 0 else jnp.maximum(mx[i], m8)
            if j == i:
                mfin[i] = jnp.broadcast_to(jnp.max(mx[i], axis=0, keepdims=True), (8, T))

        def pv(n):
            i, j = tiles[n]
            m = mfin[i]
            if hist:
                dep = hist[-1]
                if n + AH < NTL and len(seen) > n + AH + 4:
                    dep = jnp.maximum(dep, seen[n + AH])
                m = jnp.where(dep < 0, dep, m)
            if n in after:
                m = jnp.where(after[n] < 0, 0.0, m)
            p3 = jnp.exp2(sval.pop((i, j)).reshape(T // 8, 8, T) - m[None])
            l8 = jnp.sum(p3, axis=0)
            lsum[i] = l8 if j == 0 else lsum[i] + l8
            hist.append(lsum[i])
            o = _dot(_up(vt_ref[j]), p3.reshape(T, T).astype(BF))
            oacc[i] = o if j == 0 else oacc[i] + o
            if j == i:
                l = jnp.sum(lsum[i], axis=0, keepdims=True)
                ctx_ref[i * HT:(i + 1) * HT, :] = _pk((oacc[i] * (1.0 / l)).T)

        return qk, pv, after

    def out_proj(h, lo, hi):
        off = (h & 1) * HT
        off = off if isinstance(off, int) else pl.multiple_of(off, HT)
        oo = _dot(_up(ctx_ref[lo // 2:hi // 2, :]), _up(wo_ref[h >> 1, pl.ds(off, HT), :]))
        return [oo[:, t * T:(t + 1) * T] for t in range(NM)]

    def head(after_pv=None, at_t=None):
        qk, pv, _ = attention()
        for t in range(NTL + LAG):
            if t % VI == 0 and t // VI < NS:
                proj_v(t // VI)
            if at_t:
                at_t(t)
            if t < NTL:
                qk(t)
            if t >= LAG:
                pv(t - LAG)
                if after_pv:
                    after_pv(t - LAG)

    def prep(h):
        prep_k(h)
        prep_q(h)
        prep_v(h)

    (c0,), (c1,), (c2,), (c3,) = [c_copies(r) for r in range(NR)]
    x0, x1, x2, x3 = [x_copy(r) for r in range(NR)]
    for cp in [x0, w0[2], x1, x2, x3, w0[0], w0[1], c0, c1, c2, c3]:
        cp.start()
    wr = jnp.broadcast_to(wr_ref[...].reshape(1, M), (NS, M))
    sub = lax.broadcasted_iota(I32, (NS, T), 0)
    score = [jnp.zeros((NS, T), F32)]
    G = R // T

    def route(s):
        xx = jnp.concatenate([_up(xn_ref[t, s * HT:(s + 1) * HT, :]) for t in range(NM)], axis=1)
        score[0] = jnp.where(sub == s, _dot_nt(wr, xx), score[0])

    qk, pv, after = attention()
    cur = [0, 0]

    def advance(q_to, p_to):
        while cur[0] < q_to or cur[1] < p_to:
            if cur[0] < q_to:
                qk(cur[0])
                cur[0] += 1
            if cur[1] < p_to:
                pv(cur[1])
                cur[1] += 1

    for r, cps in enumerate(([x0], [w0[2], x1], [x2], [x3])):
        for cp in cps:
            cp.wait()
        if r == 1:
            prep_q(0)
        for u in range(G):
            for w in range(T // LR):
                layernorm((r * G + u) * (T // LR) + w)
                if r > 0 and w == 0:
                    proj_q((r - 1) * G + u, HT)
            if r > 0:
                route((r - 1) * G + u)
    for cp in [w0[0], w0[1], c0]:
        cp.wait()
    prep_k(0)
    prep_v(0)
    proj_q(NR - 1)
    proj_k(0)
    for s in range(G):
        route((NR - 1) * G + s)
        proj_v(s)
        advance(first(s + 1), 0)
    c1.wait()
    c2.wait()
    for cp in [w0[3]] + w_group(0):
        cp.start()
    proj_k(1)
    proj_k(2)
    for s in range(G, 2 * G):
        proj_v(s)
        advance(first(s + 1), max(first(s - G + 1), first(s + 1) - 20))
    for cp in [c3, w0[3]]:
        cp.wait()
    proj_k(3)
    for s in range(2 * G, NS):
        proj_v(s)
        advance(cur[0] + 3, cur[1])

    score = _rb(score[0])
    row8 = lax.broadcasted_iota(I32, (CAP, T), 0)
    st = dict(key=jnp.where(score != score, -jnp.inf, score), pos=sub * T + lax.broadcasted_iota(I32, (NS, T), 1),
              gate=jnp.zeros((CAP, T), F32), xs=[jnp.zeros((CAP, T), F32) for _ in range(NM)])

    def pick(i):
        key, pos = st["key"], st["pos"]
        best = jnp.max(jnp.max(key, axis=0, keepdims=True), axis=1, keepdims=True)
        cand = jnp.where(key == best, pos, S)
        sel = jnp.min(jnp.min(cand, axis=0, keepdims=True), axis=1, keepdims=True)
        hit = pos == sel
        st["key"] = jnp.where(hit, -jnp.inf, key)
        st["pos"] = jnp.where(hit, S, pos)
        st["gate"] = jnp.where(row8 == i, best, st["gate"])
        tok = jnp.minimum(sel[0, 0], S - 1)
        idx_ref[i] = tok
        after[cur[1] + 7] = sel
        for t in range(NM):
            st["xs"][t] = jnp.where(row8 == i, _half(xn_ref[t, pl.ds(tok >> 1, 1), :], tok & 1), st["xs"][t])

    npick = 0
    while cur[1] < NTL:
        lagged = cur[0] - cur[1] >= LAG or cur[0] == NTL
        advance(min(cur[0] + 1, NTL), cur[1] + lagged)
        if lagged and cur[1] % 8 == 0 and npick < CAP:
            pick(npick)
            npick += 1
    assert npick == CAP
    xs_ref[...] = jnp.concatenate(st["xs"], axis=1)
    gate = _rb(1.0 / (1.0 + jnp.exp(-st["gate"])))
    prep(1)
    for r in range(NR):
        oo = out_proj(0, r * R, (r + 1) * R)
        for t in range(NM):
            base = (x_ref[r * R:(r + 1) * R, t * T:(t + 1) * T].astype(F32)
                    + _up(xn_ref[t, r * HR:(r + 1) * HR, :]).astype(F32))
            acc_ref[t, r * R:(r + 1) * R, :] = base + oo[t]
    for cp in [wo_rest] + w_group(1) + f_copies:
        cp.start()
    for cp in w_group(0):
        cp.wait()

    def body(h, carry):
        pl.when(h == 2)(wo_rest.wait)

        @pl.when(h == 8)
        def _():
            for cp in w_group(1):
                cp.wait()

        for r in range(NR):
            proj_k(r)
        for r in range(NR):
            proj_q(r)
        head()
        prep(h + 1)
        for r in range(NR):
            oo = out_proj(h, r * R, (r + 1) * R)
            for t in range(NM):
                acc_ref[t, r * R:(r + 1) * R, :] += oo[t]
        return carry

    lax.fori_loop(1, H - 1, body, 0)

    for cp in f_copies:
        cp.wait()
    chunks = [(lo, min(lo + T, FD)) for lo in range(0, FD, T)]
    part, hid = {}, {}

    def ffn_in(k, w, t):
        lo, hi = chunks[k]
        d = _dot_nt(xs_ref[:, t * T:(t + 1) * T].astype(BF), _up(ffn_ref[w, lo // 2:hi // 2, t * T:(t + 1) * T]))
        part[k, w] = d if t == 0 else part[k, w] + d
        if w == 1 and t == NM - 1:
            g = _rb(part[k, 0])
            hid[k] = (_rb(g / (1.0 + jnp.exp(-g))) * _rb(part[k, 1])).astype(BF)

    def ffn_out(k, t):
        lo, hi = chunks[k]
        d = _dot(hid[k], _up(ffn_ref[2, lo // 2:hi // 2, t * T:(t + 1) * T]))
        part[t] = d if k == 0 else part[t] + d

    def ffn_scatter():
        for t in range(NM):
            y = _rb(_rb(part[t]) * gate)
            for i in range(CAP):
                acc_ref[t, pl.ds(idx_ref[i], 1), :] += y[i:i + 1, :]

    todo = [functools.partial(ffn_in, k, w, t) for k in range(len(chunks)) for w in range(2) for t in range(NM)]
    todo += [functools.partial(ffn_out, k, t) for k in range(len(chunks)) for t in range(NM)]
    todo += [None] * (-len(todo) % 4 + 8) + [ffn_scatter]

    def ffn_step():
        for fn in todo[:4]:
            if fn:
                fn()
        del todo[:4]

    for r in range(NR * SP):
        proj_k(r, HR // SP)
        ffn_step()
        proj_q(r, HR // SP)
        ffn_step()

    def finish(lo, hi):
        assert not todo
        oo = out_proj(H - 1, lo, hi)
        for t in range(NM):
            x_ref[lo:hi, t * T:(t + 1) * T] = (acc_ref[t, lo:hi, :] + oo[t]).astype(BF)

    outs = [o_copy(k, CUTS[k], CUTS[k + 1]) for k in range(len(CUTS) - 1)]
    plan = {}
    for lo in range(0, CUTS[-2], FC):
        hi = min(lo + FC, min(c for c in CUTS if c > lo))
        at = min(max(first(hi // T) + 8, F0 + lo // FS), NTL - 1)
        plan.setdefault(at, []).append(functools.partial(finish, lo, hi))
        if hi in CUTS:
            plan.setdefault(min(at + 6, NTL - 1), []).append(outs[CUTS.index(hi) - 1].start)
    head(lambda n: [fn() for fn in plan.get(n, ())], lambda t: ffn_step() if t % FP == 1 else None)
    assert not todo
    finish(CUTS[-2], S)
    outs[-1].start()
    for cp in outs:
        cp.wait()

@jax.jit
def pallas_parallel_sum__compressed_kv_cla__moe_arch_mod__prompt_kernel(
    A_x, A_c_kv, A_w_q, A_w_uk, A_w_uv, A_w_o, B_x, B_w_r, B_w_gate, B_w_up, B_w_down):
    B, S, M = A_x.shape
    Dc = A_c_kv.shape[2]
    H, D = A_w_q.shape[1:]
    FD = B_w_gate.shape[1]
    NP = H // 2
    hbm = pl.BlockSpec(memory_space=pltpu.HBM)
    dma = pltpu.SemaphoreType.DMA
    out = pl.pallas_call(
        functools.partial(kernel, S=S, M=M, D=D, H=H, FD=FD),
        in_specs=[hbm] * 6 + [pl.BlockSpec(memory_space=pltpu.VMEM)] + [hbm] * 3,
        out_specs=hbm,
        out_shape=jax.ShapeDtypeStruct((B, S, M), BF),
        scratch_shapes=[
            pltpu.VMEM((S, M), BF),
            pltpu.VMEM((M // T, S // 2, T), U32), pltpu.VMEM((S // 2, Dc), U32), pltpu.VMEM((M // T, S, T), F32),
            pltpu.VMEM((S // 2, D), U32), pltpu.VMEM((S // 2, D), U32), pltpu.VMEM((S // T, D // 2, T), U32),
            pltpu.VMEM((S // 2, D), U32),
            pltpu.VMEM((M, D), U32), pltpu.VMEM((Dc, D), U32), pltpu.VMEM((Dc, D), U32),
            pltpu.VMEM((2 * (M + 1), 8, D), U32), pltpu.VMEM((2 * (Dc + 1), 8, D), U32), pltpu.VMEM((2 * (Dc + 1), 8, D), U32),
            pltpu.VMEM((NP, D, M), U32),
            pltpu.VMEM((M // 2, D), U32), pltpu.VMEM((Dc // 2, D), U32), pltpu.VMEM((D // 2, Dc), U32),
            pltpu.VMEM((3, FD // 2, M), U32), pltpu.VMEM((CAP, M), F32), pltpu.SMEM((CAP,), I32),
            dma((11,)), dma((3,)), dma((S // R,)), dma((S // R,)),
        ],
        compiler_params=pltpu.CompilerParams(vmem_limit_bytes=120 * 2**20),
    )(A_x, A_c_kv, A_w_q.reshape(M, NP, 2, D), A_w_uk.reshape(Dc, NP, 2, D), A_w_uv.reshape(Dc, NP, 2, D),
      A_w_o.reshape(NP, 2 * D, M), B_w_r, B_w_gate.T, B_w_up.T, B_w_down)
    return out
```
